```python
import jax
import jax.numpy as jnp

def _softmax(x, axis=-1):
    return jax.nn.softmax(x, axis=axis)
def _gelu(x):
    return jax.nn.gelu(x, approximate=True)
def _silu(x):
    return jax.nn.silu(x)
def _sigmoid(x):
    return jax.nn.sigmoid(x)
def _layernorm(x, axis=-1, eps=1e-5):
    m = jnp.mean(x, axis=axis, keepdims=True)
    v = jnp.var(x, axis=axis, keepdims=True)
    return (x - m) / jnp.sqrt(v + eps)
def _scatter_add(tgt, idx, src, axis=0):
    return tgt.at[idx].add(src)
def _segment_sum(src, seg, n):
    return jax.ops.segment_sum(src, seg, n)
class _Rng:
    def __init__(self, key):
        self._k = key
    def _next(self):
        self._k, sub = jax.random.split(self._k)
        return sub
    def normal(self, shape):
        return jax.random.normal(self._next(), shape, dtype=jnp.bfloat16)
    def randint(self, lo, hi, shape):
        return jax.random.randint(self._next(), shape, lo, hi, dtype=jnp.int32)
    def uniform(self, shape, lo=0.0, hi=1.0):
        return jax.random.uniform(self._next(), shape, jnp.bfloat16, lo, hi)
    def permutation(self, n):
        return jax.random.permutation(self._next(), n)


kernel_name = 'gated_mix__linear_attn_block__moe_arch_mod__prompt'

def setup_inputs():
    _rng = _Rng(jax.random.key(int.from_bytes(__import__("os").urandom(4), "little")))
    _w = (lambda a: (lambda t: t.astype(jnp.bfloat16) if jnp.issubdtype(t.dtype, jnp.floating) else t)(jnp.asarray(a)))
    def _A_setup():
        B, S, D = 1, 2048, 1024
        return {
            "x": _w((lambda *s: _rng.normal(s) * 0.05)(B, S, D)),
            "wqkv": _w((lambda *s: _rng.normal(s) * 0.05)(D, 3 * D)),
            "wo": _w((lambda *s: _rng.normal(s) * 0.05)(D, D)),
        }
    _A_in = _A_setup()

    def _B_setup():
        B, S, D, F, C = 1, 2048, 1024, 3584, 1
        return {
            "x": _w((lambda *s: _rng.normal(s) * 0.05)(B, S, D)),
            "w_r": _w((lambda *s: _rng.normal(s) * 0.05)(D)),
            "w_gate": _w((lambda *s: _rng.normal(s) * 0.05)(D, F)),
            "w_up": _w((lambda *s: _rng.normal(s) * 0.05)(D, F)),
            "w_down": _w((lambda *s: _rng.normal(s) * 0.05)(F, D)),
        }
    _B_in = _B_setup()

    return {
        "A_x": _A_in["x"],
        "A_wqkv": _A_in["wqkv"],
        "A_wo": _A_in["wo"],
        "B_x": _B_in["x"],
        "B_w_r": _B_in["w_r"],
        "B_w_gate": _B_in["w_gate"],
        "B_w_up": _B_in["w_up"],
        "B_w_down": _B_in["w_down"],
        "gate_w": _w((lambda *s: _rng.normal(s) * 0.05)(1024)),
    }

def reference(A_x, A_wqkv, A_wo, B_x, B_w_r, B_w_gate, B_w_up, B_w_down, gate_w):
    def _A_ref(x, wqkv, wo):
        B, S, D = x.shape
        H = 32; Dh = D // H
        qkv = (lambda x, *d: x.transpose(*d))((x @ wqkv).reshape(B, S, 3, H, Dh), 2, 0, 3, 1, 4)
        q, k, v = qkv[0], qkv[1], qkv[2]
        phi = lambda t: jnp.where(t > 0, t + 1, jnp.exp(t)) + 1e-6
        pq, pk = phi(q), phi(k)
        kv = jnp.einsum("bhsd,bhse->bhde", pk, v)
        z = jnp.einsum("bhsd->bhd", pk)
        num = jnp.einsum("bhqd,bhde->bhqe", pq, kv)
        den = jnp.einsum("bhqd,bhd->bhq", pq, z)[..., None] + 1e-6
        o = num / den
        return (lambda x, *d: x.transpose(*d))(o, 0, 2, 1, 3).reshape(B, S, D) @ wo

    def _B_ref(x, w_r, w_gate, w_up, w_down):
        B, S, D = x.shape
        C = 1
        r = x @ w_r
        idx = jnp.argsort(-r, axis=-1)[:, :C]
        idx_e = jnp.repeat(idx.reshape(B, C, 1), D, axis=2)
        x_sel = jnp.take_along_axis(x, idx_e, axis=1)
        g = _silu(x_sel @ w_gate)
        u = x_sel @ w_up
        y = (g * u) @ w_down
        r_sel = _sigmoid(jnp.take_along_axis(r, idx, axis=1))
        y = y * r_sel.reshape(B, C, 1)
        b_off = (jnp.arange(B) * S).reshape(B, 1)
        flat_idx = (idx + b_off).reshape(B * C)
        zero = (x * 0.0).reshape(B * S, D)
        upd = _scatter_add(zero, flat_idx, y.reshape(B * C, D), axis=0)
        return x + upd.reshape(B, S, D)

    x = A_x
    g = _sigmoid((x * gate_w).sum(-1, keepdims=True))
    a = _A_ref(x, A_wqkv, A_wo)
    b = _B_ref(x, B_w_r, B_w_gate, B_w_up, B_w_down)
    return g * a + (1 - g) * b
```

```python
import jax
import jax.numpy as jnp
from jax import lax
import jax.experimental.pallas as pl
import jax.experimental.pallas.tpu as pltpu

CFG = dict(SC=512, KA=256, FFN=1, NQ=128, NT=128, MK=512, MT=512, NA=128, MQ=512, MA=512, KS=1024)

S, D, F, DH = 2048, 1024, 3584, 32
F32, BF16 = jnp.float32, jnp.bfloat16
NT = (((1,), (1,)), ((), ()))


def _phi(t):
    return jnp.where(t > 0, t + 1.0, jnp.exp(t)) + 1e-6


def _sigmoid(t):
    return 1.0 / (1.0 + jnp.exp(-t))


def _wide(ref, rows):
    return jnp.concatenate([ref[k, rows, :] for k in range(ref.shape[0])], axis=1)


def _put_wide(ref, rows, k0, val):
    for k in range(val.shape[1] // 128):
        ref[k0 + k, rows, :] = val[:, k * 128:(k + 1) * 128]


def _body(x_hbm, wqkv_hbm, wo_hbm, wr_ref, wg_hbm, wu_hbm, wd_hbm, gw_ref, out_hbm,
          x_v, wka_v, wkb_v, wq_v, wv_v, wo_v, wg_v, wu_v, wd_v,
          wt_v, t_v, z_v, m_v, r_v, g_v, pk_v, pqn_v, xs_v, h_v, y_v, out_v,
          sem_x, sem_w, sem_f, sem_o):
    SC, KA = CFG['SC'], CFG['KA']
    NC = S // SC
    NF = wg_v.shape[0]
    FC = F // NF

    def x_cp(c):
        return pltpu.make_async_copy(x_hbm.at[pl.ds(c * SC, SC)], x_v.at[pl.ds(c * SC, SC)], sem_x.at[c])

    wq_cp = pltpu.make_async_copy(wqkv_hbm.at[:, pl.ds(0, D)], wq_v, sem_w.at[0])
    wka_cp = pltpu.make_async_copy(wqkv_hbm.at[:, pl.ds(D, KA)], wka_v, sem_w.at[1])
    wkb_cp = pltpu.make_async_copy(wqkv_hbm.at[:, pl.ds(D + KA, D - KA)], wkb_v, sem_w.at[2])
    wv_cp = pltpu.make_async_copy(wqkv_hbm.at[:, pl.ds(2 * D, D)], wv_v, sem_w.at[3])
    wo_cp = pltpu.make_async_copy(wo_hbm, wo_v, sem_w.at[4])

    def f_cps(i):
        o = pl.multiple_of(i * FC, 128)
        return (pltpu.make_async_copy(wg_hbm.at[:, pl.ds(o, FC)], wg_v.at[i], sem_f.at[0, i]),
                pltpu.make_async_copy(wu_hbm.at[:, pl.ds(o, FC)], wu_v.at[i], sem_f.at[1, i]),
                pltpu.make_async_copy(wd_hbm.at[pl.ds(o, FC)], wd_v.at[i], sem_f.at[2, i]))

    def o_cp(c):
        o = pl.multiple_of(c * SC, SC)
        return pltpu.make_async_copy(out_v.at[pl.ds(o, SC)], out_hbm.at[pl.ds(o, SC)], sem_o.at[c])

    r16 = lax.broadcasted_iota(jnp.int32, (16, D), 0)
    wr = wr_ref[...].astype(F32).reshape(1, D)
    gw = gw_ref[...].astype(F32).reshape(1, D)
    _put_wide(wt_v, slice(D, D + 16), 0,
              jnp.where(r16 == 0, wr, jnp.where(r16 == 1, gw, 0.0)).astype(BF16))

    def kt_block(m0, m1, o, first):
        NW = CFG['NT']
        MK, MT = min(CFG['MK'], m1 - m0), min(CFG['MT'], m1 - m0)
        for m in range(m0, m1, MK):
            me = min(m + MK, m1)
            rows = slice(m, me)
            zs = None if first else z_v[rows, :]
            for n in range(0, SC, 128):
                k = lax.dot_general(_wide(wt_v, slice(m, me + 16 if me == D else me)),
                                    x_v[pl.ds(o + n, 128), :], NT, preferred_element_type=F32)
                if me == D:
                    r_v[(o + n) // 128] = k[me - m:me - m + 8].astype(BF16).astype(F32)
                    g = _sigmoid(k[me - m + 1:me - m + 2])
                    g_v[pl.ds(o + n, 128), :] = jnp.broadcast_to(g, (128, 128)).T
                pk = _phi(k[:me - m])
                zs = pk if zs is None else zs + pk
                pk_v[n // 128, rows, :] = pk.astype(BF16)
            z_v[rows, :] = zs
        for m in range(m0, m1, MT):
            rows = slice(m, min(m + MT, m1))
            for n in range(0, D, NW):
                t = jnp.dot(_wide(pk_v, rows), x_v[pl.ds(o, SC), n:n + NW], preferred_element_type=F32)
                if first:
                    t_v[rows, n:n + NW] = t
                else:
                    t_v[rows, n:n + NW] += t

    x_cp(0).start()
    wka_cp.start()
    x_cp(0).wait()
    wka_cp.wait()
    wkb_cp.start()
    _put_wide(wt_v, slice(0, KA), 0, wka_v[...].T)
    kt_block(0, KA, 0, True)
    wkb_cp.wait()
    for c in range(1, NC):
        x_cp(c).start()
    wq_cp.start()
    _put_wide(wt_v, slice(KA, D), 0, wkb_v[...].T)
    kt_block(KA, D, 0, True)

    def p1(c, carry):
        x_cp(c).wait()

        @pl.when(c == 1)
        def _():
            wv_cp.start()
            wo_cp.start()

        per = -(-NF // (NC - 1))
        for t in range(per):
            i = (c - 1) * per + t - (per * (NC - 1) - NF)

            @pl.when(i >= 0)
            def _():
                for cp in f_cps(i):
                    cp.start()

        o = pl.multiple_of(c * SC, SC)
        kt_block(0, D, o, False)
        return carry

    lax.fori_loop(1, NC, p1, 0)

    wq_cp.wait()
    wv_cp.wait()
    wo_cp.wait()
    r = r_v[:, 0:1, :]
    tok = (lax.broadcasted_iota(jnp.int32, r.shape, 0) * 128
           + lax.broadcasted_iota(jnp.int32, r.shape, 2))
    best = jnp.max(jnp.max(jnp.where(r != r, -jnp.inf, r), axis=0), axis=1, keepdims=True)
    bidx = jnp.min(jnp.min(jnp.where(r == best, tok, S), axis=0), axis=1, keepdims=True)
    idx = jnp.where(bidx == S, 0, bidx)[0, 0]
    rsel = jnp.where(bidx == S, jnp.nan, best)
    c_last = idx // SC
    base = pl.multiple_of((idx // 16) * 16, 16)
    sel = lax.broadcasted_iota(jnp.int32, (16, 1), 0) == idx - base
    xsel = jnp.sum(jnp.where(sel, x_v[pl.ds(base, 16), :].astype(F32), 0.0), axis=0, keepdims=True)
    if CFG['FFN']:
        xs_v[...] = jnp.broadcast_to(xsel, (16, D)).astype(BF16)

    def ffn_steps(i):
        st = {}

        def gate(n):
            st['g'] = jnp.dot(xs_v[...], wg_v[i, :, n:n + 128], preferred_element_type=F32)

        def up(n):
            g = st['g']
            u = jnp.dot(xs_v[...], wu_v[i, :, n:n + 128], preferred_element_type=F32)
            h_v[:, n:n + 128] = (g * _sigmoid(g) * u).astype(BF16)

        def down(n):
            y_v[:, n:n + 128] += jnp.dot(h_v[...], wd_v[i, :, n:n + 128], preferred_element_type=F32)

        steps = []
        if CFG['FFN']:
            for n in range(0, FC, 128):
                steps += [(gate, n), (up, n)]
            steps += [(down, n) for n in range(0, D, 128)]
        return steps

    def qa_part(c, last, steps):
        NQ, NA, MQ, MA = CFG['NQ'], CFG['NA'], CFG['MQ'], CFG['MA']
        steps = list(steps)

        nslots = [(SC // NQ) * (D // MQ) + (SC // MA) * (D // NA)]

        def fill():
            for _ in range(-(-len(steps) // nslots[0])):
                fn, n = steps.pop(0)
                fn(n)
            nslots[0] -= 1

        o = pl.multiple_of(c * SC, SC)
        for n in range(0, SC, NQ):
            for m in range(0, D, MQ):
                fill()
                q = lax.dot_general(_wide(wt_v, slice(m, m + MQ)), x_v[pl.ds(o + n, NQ), :], NT,
                                    preferred_element_type=F32)
                pq = _phi(q)
                zz = jnp.tile(z_v[m:m + MQ, :], (1, NQ // 128))
                den = jnp.sum((pq * zz).reshape(MQ // DH, DH, NQ), axis=1, keepdims=True) + 1e-6
                p = (pq.reshape(MQ // DH, DH, NQ) * (1.0 / den)).reshape(MQ, NQ)
                _put_wide(pqn_v, slice(n, n + NQ), m // 128, p.T.astype(BF16))
        for m in range(0, SC, MA):
            for n in range(0, D, NA):
                fill()
                g = jnp.tile(g_v[pl.ds(o + m, MA), :], (1, NA // 128))
                a = jnp.dot(_wide(pqn_v, slice(m, m + MA)),
                            _wide(m_v.at[n // 128:(n + NA) // 128], slice(None)), preferred_element_type=F32)
                b = x_v[pl.ds(o + m, MA), n:n + NA].astype(F32)
                if last:
                    t_v[m:m + MA, n:n + NA] = a
                out_v[pl.ds(o + m, MA), n:n + NA] = (g * a + (1.0 - g) * (b + b * 0.0)).astype(BF16)
        if last:
            y = y_v[...] * _sigmoid(rsel)
            a = t_v[pl.ds(pl.multiple_of(base - o, 16), 16), :]
            g = jnp.tile(g_v[pl.ds(base, 16), :], (1, D // 128))
            b = x_v[pl.ds(base, 16), :].astype(F32)
            upd = b * 0.0 + jnp.where(sel, y, 0.0)
            out_v[pl.ds(base, 16), :] = (g * a + (1.0 - g) * (b + upd)).astype(BF16)
        o_cp(c).start()

    _put_wide(wt_v, slice(0, D), 0, wq_v[...].T)
    z_v[...] = jnp.broadcast_to(jnp.sum(z_v[...], axis=1, keepdims=True), z_v.shape)
    hr = lax.broadcasted_iota(jnp.int32, (128, 128), 0) // DH
    hc = lax.broadcasted_iota(jnp.int32, (128, 128), 1) // DH
    for j in range(D // 128):
        sl = slice(j * 128, (j + 1) * 128)
        kv = jnp.dot(t_v[sl, :].astype(BF16), wv_v[:, sl], preferred_element_type=F32)
        kv = jnp.where(hr == hc, kv, 0.0).astype(BF16)
        _put_wide(m_v, sl, 0, jnp.dot(kv, wo_v[sl, :], preferred_element_type=F32).astype(BF16))
    y_v[...] = jnp.zeros_like(y_v)

    def p2(i, carry):
        for cp in f_cps(i):
            cp.wait()
        qa_part((c_last + 1 + i) % NC, False, ffn_steps(i))
        return carry

    lax.fori_loop(0, NC - 1, p2, 0)
    if NF == NC:
        for cp in f_cps(NC - 1):
            cp.wait()
    qa_part(c_last, True, ffn_steps(NC - 1) if NF == NC else [])
    for c in range(NC):
        o_cp(c).wait()


@jax.jit
def pallas_gated_mix__linear_attn_block__moe_arch_mod__prompt_kernel(
    A_x, A_wqkv, A_wo, B_x, B_w_r, B_w_gate, B_w_up, B_w_down, gate_w,
):
    del B_x
    SC, KA = CFG['SC'], CFG['KA']
    NC = S // SC
    NF = NC if (F // 128) % NC == 0 else NC - 1
    FC = F // NF
    hbm = pl.BlockSpec(memory_space=pl.ANY)
    vmem = pl.BlockSpec(memory_space=pltpu.VMEM)
    out = pl.pallas_call(
        _body,
        out_shape=jax.ShapeDtypeStruct((S, D), BF16),
        in_specs=[hbm, hbm, hbm, vmem, hbm, hbm, hbm, vmem],
        out_specs=hbm,
        scratch_shapes=[
            pltpu.VMEM((S, D), BF16),
            pltpu.VMEM((D, KA), BF16),
            pltpu.VMEM((D, D - KA), BF16),
            pltpu.VMEM((D, D), BF16),
            pltpu.VMEM((D, D), BF16),
            pltpu.VMEM((D, D), BF16),
            pltpu.VMEM((NF, D, FC), BF16),
            pltpu.VMEM((NF, D, FC), BF16),
            pltpu.VMEM((NF, FC, D), BF16),
            pltpu.VMEM((D // 128, D + 16, 128), BF16),
            pltpu.VMEM((D, D), F32),
            pltpu.VMEM((D, 128), F32),
            pltpu.VMEM((D // 128, D, 128), BF16),
            pltpu.VMEM((S // 128, 8, 128), F32),
            pltpu.VMEM((S, 128), F32),
            pltpu.VMEM((SC // 128, D, 128), BF16),
            pltpu.VMEM((D // 128, SC, 128), BF16),
            pltpu.VMEM((16, D), BF16),
            pltpu.VMEM((16, FC), BF16),
            pltpu.VMEM((16, D), F32),
            pltpu.VMEM((S, D), BF16),
            pltpu.SemaphoreType.DMA((NC,)),
            pltpu.SemaphoreType.DMA((5,)),
            pltpu.SemaphoreType.DMA((3, NF)),
            pltpu.SemaphoreType.DMA((NC,)),
        ],
        compiler_params=pltpu.CompilerParams(vmem_limit_bytes=100 * 1024 * 1024),
    )(A_x.reshape(S, D), A_wqkv, A_wo, B_w_r, B_w_gate, B_w_up, B_w_down, gate_w)
    return out.reshape(1, S, D)
```

```python
import jax
import jax.numpy as jnp
from jax import lax
import jax.experimental.pallas as pl
import jax.experimental.pallas.tpu as pltpu

CFG = dict(SC=512, KA=256, FFN=1, NQ=128, NT=128, MK=512, MT=512, NA=128, MQ=512, MA=256, U1=1, U2=1)

S, D, F, DH = 2048, 1024, 3584, 32
F32, BF16 = jnp.float32, jnp.bfloat16
NT = (((1,), (1,)), ((), ()))


def _phi(t):
    return jnp.where(t > 0, t + 1.0, jnp.exp(t)) + 1e-6


def _sigmoid(t):
    return 1.0 / (1.0 + jnp.exp(-t))


def _wide(ref, rows):
    return jnp.concatenate([ref[k, rows, :] for k in range(ref.shape[0])], axis=1)


def _put_wide(ref, rows, k0, val):
    for k in range(val.shape[1] // 128):
        ref[k0 + k, rows, :] = val[:, k * 128:(k + 1) * 128]


def _body(x_hbm, wqkv_hbm, wo_hbm, wr_ref, wg_hbm, wu_hbm, wd_hbm, gw_ref, out_hbm,
          x_v, wka_v, wkb_v, wq_v, wv_v, wo_v, wg_v, wu_v, wd_v,
          wt_v, t_v, z_v, m_v, r_v, g_v, pk_v, pqn_v, xs_v, y_v, out_v,
          sem_x, sem_w, sem_f, sem_o):
    SC, KA, MA = CFG['SC'], CFG['KA'], CFG['MA']
    NC = S // SC
    NF = wg_v.shape[0]
    FC = F // NF

    def x_cp(c):
        return pltpu.make_async_copy(x_hbm.at[pl.ds(c * SC, SC)], x_v.at[pl.ds(c * SC, SC)], sem_x.at[c])

    wq_cp = pltpu.make_async_copy(wqkv_hbm.at[:, pl.ds(0, D)], wq_v, sem_w.at[0])
    wka_cp = pltpu.make_async_copy(wqkv_hbm.at[:, pl.ds(D, KA)], wka_v, sem_w.at[1])
    wkb_cp = pltpu.make_async_copy(wqkv_hbm.at[:, pl.ds(D + KA, D - KA)], wkb_v, sem_w.at[2])
    wv_cp = pltpu.make_async_copy(wqkv_hbm.at[:, pl.ds(2 * D, D)], wv_v, sem_w.at[3])
    wo_cp = pltpu.make_async_copy(wo_hbm, wo_v, sem_w.at[4])

    def f_cps(i):
        o = i * FC
        return (pltpu.make_async_copy(wg_hbm.at[:, pl.ds(o, FC)], wg_v.at[i], sem_f.at[0, i]),
                pltpu.make_async_copy(wu_hbm.at[:, pl.ds(o, FC)], wu_v.at[i], sem_f.at[1, i]),
                pltpu.make_async_copy(wd_hbm.at[pl.ds(o, FC)], wd_v.at[i], sem_f.at[2, i]))

    def o_cp(j):
        o = pl.multiple_of(j * MA, MA)
        return pltpu.make_async_copy(out_v.at[pl.ds(o, MA)], out_hbm.at[pl.ds(o, MA)], sem_o.at[j])

    r16 = lax.broadcasted_iota(jnp.int32, (16, D), 0)
    wr = wr_ref[...].astype(F32).reshape(1, D)
    gw = gw_ref[...].astype(F32).reshape(1, D)
    _put_wide(wt_v, slice(D, D + 16), 0,
              jnp.where(r16 == 0, wr, jnp.where(r16 == 1, gw, 0.0)).astype(BF16))

    def kt_block(m0, m1, o, first, between=None):
        NW = CFG['NT']
        MK, MT = min(CFG['MK'], m1 - m0), min(CFG['MT'], m1 - m0)
        for m in range(m0, m1, MK):
            me = min(m + MK, m1)
            rows = slice(m, me)
            zs = None if first else z_v[rows, :]
            for n in range(0, SC, 128):
                k = lax.dot_general(_wide(wt_v, slice(m, me + 16 if me == D else me)),
                                    x_v[pl.ds(o + n, 128), :], NT, preferred_element_type=F32)
                if me == D:
                    r_v[(o + n) // 128] = k[me - m:me - m + 8].astype(BF16).astype(F32)
                    g = _sigmoid(k[me - m + 1:me - m + 2])
                    g_v[pl.ds(o + n, 128), :] = jnp.broadcast_to(g, (128, 128)).T
                pk = _phi(k[:me - m])
                zs = pk if zs is None else zs + pk
                pk_v[n // 128, rows, :] = pk.astype(BF16)
            z_v[rows, :] = zs
        if between is not None:
            between()
        for m in range(m0, m1, MT):
            rows = slice(m, min(m + MT, m1))
            for n in range(0, D, NW):
                t = jnp.dot(_wide(pk_v, rows), x_v[pl.ds(o, SC), n:n + NW], preferred_element_type=F32)
                if first:
                    t_v[rows, n:n + NW] = t
                else:
                    t_v[rows, n:n + NW] += t

    x_cp(0).start()
    wka_cp.start()
    x_cp(0).wait()
    wka_cp.wait()
    wkb_cp.start()
    _put_wide(wt_v, slice(0, KA), 0, wka_v[...].T)
    kt_block(0, KA, 0, True)
    wkb_cp.wait()
    for c in range(1, NC):
        x_cp(c).start()
    _put_wide(wt_v, slice(KA, D), 0, wkb_v[...].T)

    def start_rest():
        for cp in (wq_cp, wv_cp, wo_cp):
            cp.start()
        for i in range(NF):
            for cp in f_cps(i):
                cp.start()

    kt_block(KA, D, 0, True, start_rest)
    for c in range(1, NC):
        x_cp(c).wait()

    def p1(c, carry):
        kt_block(0, D, pl.multiple_of(c * SC, SC), False)
        return carry

    lax.fori_loop(1, NC, p1, 0)

    wq_cp.wait()
    wv_cp.wait()
    wo_cp.wait()
    for i in range(NF):
        for cp in f_cps(i):
            cp.wait()
    r = r_v[:, 0:1, :]
    tok = (lax.broadcasted_iota(jnp.int32, r.shape, 0) * 128
           + lax.broadcasted_iota(jnp.int32, r.shape, 2))
    best = jnp.max(jnp.max(jnp.where(r != r, -jnp.inf, r), axis=0), axis=1, keepdims=True)
    bidx = jnp.min(jnp.min(jnp.where(r == best, tok, S), axis=0), axis=1, keepdims=True)
    idx = jnp.where(bidx == S, 0, bidx)[0, 0]
    rsel = jnp.where(bidx == S, jnp.nan, best)
    c_last = idx // SC
    base = pl.multiple_of((idx // 16) * 16, 16)
    sel = lax.broadcasted_iota(jnp.int32, (16, 1), 0) == idx - base
    xsel = jnp.sum(jnp.where(sel, x_v[pl.ds(base, 16), :].astype(F32), 0.0), axis=0, keepdims=True)
    xs_v[...] = jnp.broadcast_to(xsel, (8, D))

    def ffn_steps(i):
        st = {}
        HK = D // 2

        def proj(key, w_v, n, k):
            def step():
                p = lax.dot_general(xs_v[:, k:k + HK], w_v[i, k:k + HK, n:n + 128], (((1,), (0,)), ((), ())), preferred_element_type=F32)
                st[key] = p if k == 0 else st[key] + p
            return step

        def down(n, k):
            def step():
                if k == 0:
                    g = st['g']
                    st['h'] = (g * _sigmoid(g) * st['u']).astype(BF16).astype(F32)
                y_v[:, k:k + HK] += lax.dot_general(st['h'], wd_v[i, n:n + 128, k:k + HK], (((1,), (0,)), ((), ())), preferred_element_type=F32)
            return step

        steps = []
        for n in range(0, FC, 128):
            steps += [proj('g', wg_v, n, 0), proj('g', wg_v, n, HK), proj('u', wu_v, n, 0), proj('u', wu_v, n, HK)]
            if n:
                steps += [down(n - 128, 0), down(n - 128, HK)]
                steps[-6:] = [steps[-2], steps[-6], steps[-1]] + steps[-5:-2]
        return steps + [down(FC - 128, 0), down(FC - 128, HK)]

    def qa_part(c, steps, more):
        NQ, NA, MQ = CFG['NQ'], CFG['NA'], CFG['MQ']
        HK = D // 2
        steps = list(steps)

        def fill():
            if steps:
                steps.pop(0)()

        o = pl.multiple_of(c * SC, SC)
        for n in range(0, SC, NQ):
            for m in range(0, D, MQ):
                q = None
                for k in range(0, D, HK):
                    fill()
                    p = lax.dot_general(_wide(wt_v.at[k // 128:(k + HK) // 128], slice(m, m + MQ)),
                                        x_v[pl.ds(o + n, NQ), k:k + HK], NT, preferred_element_type=F32)
                    q = p if q is None else q + p
                pq = _phi(q)
                zz = jnp.tile(z_v[m:m + MQ, :], (1, NQ // 128))
                den = jnp.sum((pq * zz).reshape(MQ // DH, DH, NQ), axis=1, keepdims=True) + 1e-6
                p = (pq.reshape(MQ // DH, DH, NQ) * (1.0 / den)).reshape(MQ, NQ)
                _put_wide(pqn_v, slice(n, n + NQ), m // 128, p.T.astype(BF16))
        NB = SC // MA
        for t in range(NB):
            j = (idx // MA + 1 + t) % NB
            m = pl.multiple_of(j * MA, MA)
            for n in range(0, D, NA):
                a = None
                for k in range(0, D, HK):
                    fill()
                    p = jnp.dot(_wide(pqn_v.at[k // 128:(k + HK) // 128], pl.ds(m, MA)),
                                _wide(m_v.at[n // 128:(n + NA) // 128], slice(k, k + HK)),
                                preferred_element_type=F32)
                    a = p if a is None else a + p
                g = jnp.tile(g_v[pl.ds(o + m, MA), :], (1, NA // 128))
                b = x_v[pl.ds(o + m, MA), n:n + NA].astype(F32)
                if t == NB - 1:
                    t_v[:MA, n:n + NA] = a
                out_v[pl.ds(o + m, MA), n:n + NA] = (g * a + (1.0 - g) * (b + b * 0.0)).astype(BF16)
            if t < NB - 1:
                o_cp(c * NB + j).start()
            else:
                pl.when(more)(o_cp(c * NB + j).start)
        assert not steps

    _put_wide(wt_v, slice(0, D), 0, wq_v[...].T)
    z_v[...] = jnp.broadcast_to(jnp.sum(z_v[...], axis=1, keepdims=True), z_v.shape)
    hr = lax.broadcasted_iota(jnp.int32, (128, 128), 0) // DH
    hc = lax.broadcasted_iota(jnp.int32, (128, 128), 1) // DH
    for j in range(D // 128):
        sl = slice(j * 128, (j + 1) * 128)
        kv = jnp.dot(t_v[sl, :].astype(BF16), wv_v[:, sl], preferred_element_type=F32)
        kv = jnp.where(hr == hc, kv, 0.0).astype(BF16)
        _put_wide(m_v, sl, 0, jnp.dot(kv, wo_v[sl, :], preferred_element_type=F32).astype(BF16))
    y_v[...] = jnp.zeros_like(y_v)

    def p2(i, carry):
        qa_part((c_last + 1 + i) % NC, ffn_steps(i), i < NC - 1)
        return carry

    lax.fori_loop(0, NC, p2, 0)

    y = y_v[:1, :] * _sigmoid(rsel)
    a = t_v[pl.ds(pl.multiple_of(base % MA, 16), 16), :]
    g = jnp.tile(g_v[pl.ds(base, 16), :], (1, D // 128))
    b = x_v[pl.ds(base, 16), :].astype(F32)
    upd = b * 0.0 + jnp.where(sel, y, 0.0)
    out_v[pl.ds(base, 16), :] = (g * a + (1.0 - g) * (b + upd)).astype(BF16)
    o_cp(idx // MA).start()
    for j in range(S // MA):
        o_cp(j).wait()


@jax.jit
def pallas_gated_mix__linear_attn_block__moe_arch_mod__prompt_kernel(
    A_x, A_wqkv, A_wo, B_x, B_w_r, B_w_gate, B_w_up, B_w_down, gate_w,
):
    del B_x
    SC, KA = CFG['SC'], CFG['KA']
    NC = S // SC
    NF = NC
    FC = F // NF
    hbm = pl.BlockSpec(memory_space=pl.ANY)
    vmem = pl.BlockSpec(memory_space=pltpu.VMEM)
    out = pl.pallas_call(
        _body,
        out_shape=jax.ShapeDtypeStruct((S, D), BF16),
        in_specs=[hbm, hbm, hbm, vmem, hbm, hbm, hbm, vmem],
        out_specs=hbm,
        scratch_shapes=[
            pltpu.VMEM((S, D), BF16),
            pltpu.VMEM((D, KA), BF16),
            pltpu.VMEM((D, D - KA), BF16),
            pltpu.VMEM((D, D), BF16),
            pltpu.VMEM((D, D), BF16),
            pltpu.VMEM((D, D), BF16),
            pltpu.VMEM((NF, D, FC), BF16),
            pltpu.VMEM((NF, D, FC), BF16),
            pltpu.VMEM((NF, FC, D), BF16),
            pltpu.VMEM((D // 128, D + 16, 128), BF16),
            pltpu.VMEM((D, D), F32),
            pltpu.VMEM((D, 128), F32),
            pltpu.VMEM((D // 128, D, 128), BF16),
            pltpu.VMEM((S // 128, 8, 128), F32),
            pltpu.VMEM((S, 128), F32),
            pltpu.VMEM((SC // 128, D, 128), BF16),
            pltpu.VMEM((D // 128, SC, 128), BF16),
            pltpu.VMEM((8, D), F32),
            pltpu.VMEM((8, D), F32),
            pltpu.VMEM((S, D), BF16),
            pltpu.SemaphoreType.DMA((NC,)),
            pltpu.SemaphoreType.DMA((5,)),
            pltpu.SemaphoreType.DMA((3, NF)),
            pltpu.SemaphoreType.DMA((S // CFG['MA'],)),
        ],
        compiler_params=pltpu.CompilerParams(vmem_limit_bytes=100 * 1024 * 1024),
    )(A_x.reshape(S, D), A_wqkv, A_wo, B_w_r, B_w_gate, B_w_up, B_w_down, gate_w)
    return out.reshape(1, S, D)
```

```python
import jax
import jax.numpy as jnp
from jax import lax
import jax.experimental.pallas as pl
import jax.experimental.pallas.tpu as pltpu

CFG = dict(SC=512, KA=256, FFN=1, NQ=128, NT=128, MK=512, MT=512, NA=128, MQ=512, MA=256, TN=6, HN=0)

S, D, F, DH = 2048, 1024, 3584, 32
F32, BF16 = jnp.float32, jnp.bfloat16
NT = (((1,), (1,)), ((), ()))


def _phi(t):
    return jnp.where(t > 0, t + 1.0, jnp.exp(t)) + 1e-6


def _sigmoid(t):
    return 1.0 / (1.0 + jnp.exp(-t))


def _wide(ref, rows):
    return jnp.concatenate([ref[k, rows, :] for k in range(ref.shape[0])], axis=1)


def _put_wide(ref, rows, k0, val):
    for k in range(val.shape[1] // 128):
        ref[k0 + k, rows, :] = val[:, k * 128:(k + 1) * 128]


def _body(x_hbm, wqkv_hbm, wo_hbm, wr_ref, wg_hbm, wu_hbm, wd_hbm, gw_ref, out_hbm,
          x_v, wka_v, wkb_v, wq_v, wv_v, wo_v, wg_v, wu_v, wd_v,
          wt_v, t_v, z_v, m_v, r_v, g_v, pk_v, pqn_v, xs_v, y_v, out_v,
          sem_x, sem_w, sem_f, sem_o):
    SC, KA, MA = CFG['SC'], CFG['KA'], CFG['MA']
    NC = S // SC
    NF = wg_v.shape[0]
    FC = F // NF

    def x_cp(c):
        return pltpu.make_async_copy(x_hbm.at[pl.ds(c * SC, SC)], x_v.at[pl.ds(c * SC, SC)], sem_x.at[c])

    wq_cp = pltpu.make_async_copy(wqkv_hbm.at[:, pl.ds(0, D)], wq_v, sem_w.at[0])
    wka_cp = pltpu.make_async_copy(wqkv_hbm.at[:, pl.ds(D, KA)], wka_v, sem_w.at[1])
    wkb_cp = pltpu.make_async_copy(wqkv_hbm.at[:, pl.ds(D + KA, D - KA)], wkb_v, sem_w.at[2])
    wv_cp = pltpu.make_async_copy(wqkv_hbm.at[:, pl.ds(2 * D, D)], wv_v, sem_w.at[3])
    wo_cp = pltpu.make_async_copy(wo_hbm, wo_v, sem_w.at[4])

    def f_cps(i):
        o = i * FC
        return (pltpu.make_async_copy(wg_hbm.at[:, pl.ds(o, FC)], wg_v.at[i], sem_f.at[0, i]),
                pltpu.make_async_copy(wu_hbm.at[:, pl.ds(o, FC)], wu_v.at[i], sem_f.at[1, i]),
                pltpu.make_async_copy(wd_hbm.at[pl.ds(o, FC)], wd_v.at[i], sem_f.at[2, i]))

    def o_cp(j):
        o = pl.multiple_of(j * MA, MA)
        return pltpu.make_async_copy(out_v.at[pl.ds(o, MA)], out_hbm.at[pl.ds(o, MA)], sem_o.at[j])

    r16 = lax.broadcasted_iota(jnp.int32, (16, D), 0)
    wr = wr_ref[...].astype(F32).reshape(1, D)
    gw = gw_ref[...].astype(F32).reshape(1, D)
    _put_wide(wt_v, slice(D, D + 16), 0,
              jnp.where(r16 == 0, wr, jnp.where(r16 == 1, gw, 0.0)).astype(BF16))

    def kt_block(m0, m1, o, first, between=None):
        NW = CFG['NT']
        MK, MT = min(CFG['MK'], m1 - m0), min(CFG['MT'], m1 - m0)
        for m in range(m0, m1, MK):
            me = min(m + MK, m1)
            rows = slice(m, me)
            zs = None if first else z_v[rows, :]
            for n in range(0, SC, 128):
                k = lax.dot_general(_wide(wt_v, slice(m, me + 16 if me == D else me)),
                                    x_v[pl.ds(o + n, 128), :], NT, preferred_element_type=F32)
                if me == D:
                    r_v[(o + n) // 128] = k[me - m:me - m + 8].astype(BF16).astype(F32)
                    g = _sigmoid(k[me - m + 1:me - m + 2])
                    g_v[pl.ds(o + n, 128), :] = jnp.broadcast_to(g, (128, 128)).T
                pk = _phi(k[:me - m])
                zs = pk if zs is None else zs + pk
                pk_v[n // 128, rows, :] = pk.astype(BF16)
            z_v[rows, :] = zs
        if between is not None:
            between()
        for m in range(m0, m1, MT):
            rows = slice(m, min(m + MT, m1))
            for n in range(0, D, NW):
                t = jnp.dot(_wide(pk_v, rows), x_v[pl.ds(o, SC), n:n + NW], preferred_element_type=F32)
                if first:
                    t_v[rows, n:n + NW] = t
                else:
                    t_v[rows, n:n + NW] += t

    x_cp(0).start()
    wka_cp.start()
    x_cp(0).wait()
    wka_cp.wait()
    wkb_cp.start()
    _put_wide(wt_v, slice(0, KA), 0, wka_v[...].T)
    kt_block(0, KA, 0, True)
    wkb_cp.wait()
    for c in range(1, NC):
        x_cp(c).start()
    _put_wide(wt_v, slice(KA, D), 0, wkb_v[...].T)

    def start_rest():
        for cp in (wq_cp, wv_cp, wo_cp):
            cp.start()
        for i in range(NF):
            for cp in f_cps(i):
                cp.start()

    kt_block(KA, D, 0, True, start_rest)
    for c in range(1, NC):
        x_cp(c).wait()

    def p1(c, carry):
        kt_block(0, D, pl.multiple_of(c * SC, SC), False)
        return carry

    lax.fori_loop(1, NC, p1, 0)

    wq_cp.wait()
    wv_cp.wait()
    wo_cp.wait()
    for i in range(NF):
        for cp in f_cps(i):
            cp.wait()
    r = r_v[:, 0:1, :]
    tok = (lax.broadcasted_iota(jnp.int32, r.shape, 0) * 128
           + lax.broadcasted_iota(jnp.int32, r.shape, 2))
    best = jnp.max(jnp.max(jnp.where(r != r, -jnp.inf, r), axis=0), axis=1, keepdims=True)
    bidx = jnp.min(jnp.min(jnp.where(r == best, tok, S), axis=0), axis=1, keepdims=True)
    idx = jnp.where(bidx == S, 0, bidx)[0, 0]
    rsel = jnp.where(bidx == S, jnp.nan, best)
    base = pl.multiple_of((idx // 16) * 16, 16)
    sel = lax.broadcasted_iota(jnp.int32, (16, 1), 0) == idx - base
    xsel = jnp.sum(jnp.where(sel, x_v[pl.ds(base, 16), :].astype(F32), 0.0), axis=0, keepdims=True)
    xs_v[...] = jnp.broadcast_to(xsel, (8, D))

    def ffn_steps(i):
        st = {}
        HK = D // 2

        def proj(key, w_v, n, k):
            def step():
                p = lax.dot_general(xs_v[:, k:k + HK], w_v[i, k:k + HK, n:n + 128], (((1,), (0,)), ((), ())), preferred_element_type=F32)
                st[key, n] = p if k == 0 else st[key, n] + p
            return step

        def down(n, k):
            def step():
                if k == 0:
                    g = st['g', n]
                    st['h', n] = (g * _sigmoid(g) * st['u', n]).astype(BF16).astype(F32)
                y_v[:, k:k + HK] += lax.dot_general(st['h', n], wd_v[i, n:n + 128, k:k + HK], (((1,), (0,)), ((), ())), preferred_element_type=F32)
            return step

        tiles = range(0, FC, 128)
        return ([proj(key, w_v, n, k) for n in tiles for key, w_v in (('g', wg_v), ('u', wu_v)) for k in (0, HK)]
                + [down(n, k) for n in tiles for k in (0, HK)])

    def qa_part(blocks, steps, more):
        NQ, NA, MQ = CFG['NQ'], CFG['NA'], CFG['MQ']
        HK = D // 2
        steps = list(steps)

        def fill(keep=CFG['TN']):
            if len(steps) > keep:
                steps.pop(0)()

        for _ in range(CFG['HN']):
            fill()

        for n in range(0, SC, NQ):
            o = pl.multiple_of(blocks[n // MA] * MA + n % MA, NQ)
            for m in range(0, D, MQ):
                q = None
                for k in range(0, D, HK):
                    fill()
                    p = lax.dot_general(_wide(wt_v.at[k // 128:(k + HK) // 128], slice(m, m + MQ)),
                                        x_v[pl.ds(o, NQ), k:k + HK], NT, preferred_element_type=F32)
                    q = p if q is None else q + p
                pq = _phi(q)
                zz = jnp.tile(z_v[m:m + MQ, :], (1, NQ // 128))
                den = jnp.sum((pq * zz).reshape(MQ // DH, DH, NQ), axis=1, keepdims=True) + 1e-6
                p = (pq.reshape(MQ // DH, DH, NQ) * (1.0 / den)).reshape(MQ, NQ)
                _put_wide(pqn_v, slice(n, n + NQ), m // 128, p.T.astype(BF16))
        for t, j in enumerate(blocks):
            o = pl.multiple_of(j * MA, MA)
            for n in range(0, D, NA):
                a = None
                for k in range(0, D, HK):
                    fill()
                    p = jnp.dot(_wide(pqn_v.at[k // 128:(k + HK) // 128], slice(t * MA, (t + 1) * MA)),
                                _wide(m_v.at[n // 128:(n + NA) // 128], slice(k, k + HK)),
                                preferred_element_type=F32)
                    a = p if a is None else a + p
                g = jnp.tile(g_v[pl.ds(o, MA), :], (1, NA // 128))
                b = x_v[pl.ds(o, MA), n:n + NA].astype(F32)
                if t == len(blocks) - 1:
                    t_v[:MA, n:n + NA] = a
                out_v[pl.ds(o, MA), n:n + NA] = (g * a + (1.0 - g) * (b + b * 0.0)).astype(BF16)
            if t < len(blocks) - 1:
                o_cp(j).start()
            else:
                while steps:
                    fill(0)
                pl.when(more)(o_cp(j).start)
        assert not steps

    _put_wide(wt_v, slice(0, D), 0, wq_v[...].T)
    z_v[...] = jnp.broadcast_to(jnp.sum(z_v[...], axis=1, keepdims=True), z_v.shape)
    hr = lax.broadcasted_iota(jnp.int32, (128, 128), 0) // DH
    hc = lax.broadcasted_iota(jnp.int32, (128, 128), 1) // DH
    for j in range(D // 128):
        sl = slice(j * 128, (j + 1) * 128)
        kv = jnp.dot(t_v[sl, :].astype(BF16), wv_v[:, sl], preferred_element_type=F32)
        kv = jnp.where(hr == hc, kv, 0.0).astype(BF16)
        _put_wide(m_v, sl, 0, jnp.dot(kv, wo_v[sl, :], preferred_element_type=F32).astype(BF16))
    y_v[...] = jnp.zeros_like(y_v)

    def p2(i, carry):
        NB = SC // MA
        blocks = [(idx // MA + 1 + i * NB + t) % (S // MA) for t in range(NB)]
        qa_part(blocks, ffn_steps(i) if CFG['FFN'] else [], i < NC - 1)
        return carry

    lax.fori_loop(0, NC, p2, 0)

    y = y_v[:1, :] * _sigmoid(rsel)
    a = t_v[pl.ds(pl.multiple_of(base % MA, 16), 16), :]
    g = jnp.tile(g_v[pl.ds(base, 16), :], (1, D // 128))
    b = x_v[pl.ds(base, 16), :].astype(F32)
    upd = b * 0.0 + jnp.where(sel, y, 0.0)
    out_v[pl.ds(base, 16), :] = (g * a + (1.0 - g) * (b + upd)).astype(BF16)
    o_cp(idx // MA).start()
    for j in range(S // MA):
        o_cp(j).wait()


@jax.jit
def pallas_gated_mix__linear_attn_block__moe_arch_mod__prompt_kernel(
    A_x, A_wqkv, A_wo, B_x, B_w_r, B_w_gate, B_w_up, B_w_down, gate_w,
):
    del B_x
    SC, KA = CFG['SC'], CFG['KA']
    NC = S // SC
    NF = NC
    FC = F // NF
    hbm = pl.BlockSpec(memory_space=pl.ANY)
    vmem = pl.BlockSpec(memory_space=pltpu.VMEM)
    out = pl.pallas_call(
        _body,
        out_shape=jax.ShapeDtypeStruct((S, D), BF16),
        in_specs=[hbm, hbm, hbm, vmem, hbm, hbm, hbm, vmem],
        out_specs=hbm,
        scratch_shapes=[
            pltpu.VMEM((S, D), BF16),
            pltpu.VMEM((D, KA), BF16),
            pltpu.VMEM((D, D - KA), BF16),
            pltpu.VMEM((D, D), BF16),
            pltpu.VMEM((D, D), BF16),
            pltpu.VMEM((D, D), BF16),
            pltpu.VMEM((NF, D, FC), BF16),
            pltpu.VMEM((NF, D, FC), BF16),
            pltpu.VMEM((NF, FC, D), BF16),
            pltpu.VMEM((D // 128, D + 16, 128), BF16),
            pltpu.VMEM((D, D), F32),
            pltpu.VMEM((D, 128), F32),
            pltpu.VMEM((D // 128, D, 128), BF16),
            pltpu.VMEM((S // 128, 8, 128), F32),
            pltpu.VMEM((S, 128), F32),
            pltpu.VMEM((SC // 128, D, 128), BF16),
            pltpu.VMEM((D // 128, SC, 128), BF16),
            pltpu.VMEM((8, D), F32),
            pltpu.VMEM((8, D), F32),
            pltpu.VMEM((S, D), BF16),
            pltpu.SemaphoreType.DMA((NC,)),
            pltpu.SemaphoreType.DMA((5,)),
            pltpu.SemaphoreType.DMA((3, NF)),
            pltpu.SemaphoreType.DMA((S // CFG['MA'],)),
        ],
        compiler_params=pltpu.CompilerParams(vmem_limit_bytes=100 * 1024 * 1024),
    )(A_x.reshape(S, D), A_wqkv, A_wo, B_w_r, B_w_gate, B_w_up, B_w_down, gate_w)
    return out.reshape(1, S, D)
```

```python
import jax
import jax.numpy as jnp
from jax import lax
import jax.experimental.pallas as pl
import jax.experimental.pallas.tpu as pltpu

CFG = dict(FFN=1, MQ=512, MT=512)

S, D, F, DH = 2048, 1024, 3584, 32
HD = D // 2
U = 256
UH = U // 2
NU = S // U
UC = 2
NC = NU // UC
FC = F // NC
F32, BF16 = jnp.float32, jnp.bfloat16
NN = (((1,), (0,)), ((), ()))
NT = (((1,), (1,)), ((), ()))


def _dot(a, b, dims=NN):
    return lax.dot_general(a, b, dims, preferred_element_type=F32)


def _phi(t):
    return jnp.where(t > 0, t + 1.0, jnp.exp(t)) + 1e-6


def _sigmoid(t):
    return 1.0 / (1.0 + jnp.exp(-t))


def _lhs_terms(a11, a12, a21, a22):
    return [a11 + a22, a21 + a22, a11, a22, a11 + a12, a21 - a11, a12 - a22]


def _rhs_terms(b11, b12, b21, b22):
    return [b11 + b22, b11, b12 - b22, b21 - b11, b22, b11 + b12, b21 + b22]


def _combine(p):
    return p[0] + p[3] - p[4] + p[6], p[2] + p[4], p[1] + p[3], p[0] - p[1] + p[2] + p[5]


_RHS_AS_LHS = (0, 2, 6, 5, 3, 4, 1)


def _wide(ref, rows=slice(None)):
    return jnp.concatenate([ref[k, rows, :] for k in range(ref.shape[0])], axis=1)


def _put_wide(ref, rows, val):
    for k in range(val.shape[1] // 128):
        ref[k, rows, :] = val[:, k * 128:(k + 1) * 128]


def _body(x_hbm, wqkv_hbm, wo_hbm, wr_ref, wg_hbm, wu_hbm, wd_hbm, gw_ref, out_hbm,
          x_v, wk_v, wq_v, wv_v, wo_v, wg_v, wu_v, wd_v,
          xs_v, ws_v, ps_v, n_v, z_v, ms_v, rs_v, rg_v, r_v, g_v, a_v, xsel_v, y_v, out_v,
          sem_x, sem_w, sem_f, sem_o):
    MQ, MT = CFG['MQ'], CFG['MT']

    def x_cp(c):
        rows = pl.ds(c * UC * U, UC * U)
        return pltpu.make_async_copy(x_hbm.at[rows], x_v.at[rows], sem_x.at[c])

    def wk_cp(i, j):
        return pltpu.make_async_copy(wqkv_hbm.at[pl.ds(i * HD, HD), pl.ds(D + j * HD, HD)],
                                     wk_v.at[i, j], sem_w.at[2 * i + j])

    wq_cp = pltpu.make_async_copy(wqkv_hbm.at[:, pl.ds(0, D)], wq_v, sem_w.at[4])
    wv_cp = pltpu.make_async_copy(wqkv_hbm.at[:, pl.ds(2 * D, D)], wv_v, sem_w.at[5])
    wo_cp = pltpu.make_async_copy(wo_hbm, wo_v, sem_w.at[6])

    def f_cps(i):
        return (pltpu.make_async_copy(wg_hbm.at[:, pl.ds(i * FC, FC)], wg_v.at[i], sem_f.at[0, i]),
                pltpu.make_async_copy(wu_hbm.at[:, pl.ds(i * FC, FC)], wu_v.at[i], sem_f.at[1, i]),
                pltpu.make_async_copy(wd_hbm.at[pl.ds(i * FC, FC)], wd_v.at[i], sem_f.at[2, i]))

    def o_cp(u):
        rows = pl.ds(pl.multiple_of(u * U, U), U)
        return pltpu.make_async_copy(out_v.at[rows], out_hbm.at[rows], sem_o.at[u])

    def x_quadrant(u, i, j):
        return x_v[pl.ds(pl.multiple_of(u * U + i * UH, UH), UH), j * HD:(j + 1) * HD]

    def make_x_terms(u):
        t = _lhs_terms(*[x_quadrant(u, i, j).astype(F32) for i in (0, 1) for j in (0, 1)])
        for slot, i in enumerate((0, 1, 4, 5, 6)):
            xs_v[slot, pl.ds(pl.multiple_of(u * UH, UH), UH), :] = t[i].astype(BF16)

    def x_term(u, i):
        if i in (2, 3):
            return x_quadrant(u, i - 2, i - 2)
        return xs_v[(0, 1, None, None, 2, 3, 4)[i], pl.ds(pl.multiple_of(u * UH, UH), UH), :]

    def put_w_terms(which, wt):
        f = [None if w is None else w.astype(F32) for w in wt]
        for i in which:
            if i in (1, 4):
                t = wt[0 if i == 1 else 3]
            else:
                a, b, sign = {0: (0, 3, 1), 2: (1, 3, -1), 3: (2, 0, -1), 5: (0, 1, 1), 6: (2, 3, 1)}[i]
                t = (f[a] + f[b] if sign > 0 else f[a] - f[b]).astype(BF16)
            _put_wide(ws_v.at[i], slice(None), t)

    def proj_term(u, i, rows):
        return _dot(_wide(ws_v.at[i], rows), x_term(u, i), NT)

    def route(u):
        for h in range(2):
            o = pl.multiple_of(u * U + h * UH, UH)
            rg = _dot(rg_v[...], x_v[pl.ds(o, UH), :], NT)
            r_v[2 * u + h] = rg[:8].astype(BF16).astype(F32)
            g_v[pl.ds(o, UH), :] = jnp.broadcast_to(_sigmoid(rg[1:2]), (UH, UH)).T

    def k_finish(t, rows, prods, first):
        k11, k12, k21, k22 = [_phi(k) for k in _combine(prods)]
        lo, hi = rows, slice(HD + rows.start, HD + rows.stop)
        if first:
            z_v[lo, :] = k11 + k21
            z_v[hi, :] = k12 + k22
        else:
            z_v[lo, :] += k11 + k21
            z_v[hi, :] += k12 + k22
        for i, p in enumerate(_lhs_terms(k11, k21, k12, k22)):
            ps_v[i, t, rows, :] = p.astype(BF16)

    def t_part(units, first):
        for i in (1, 4, 0, 2, 3, 5, 6):
            for m in range(0, HD, MT):
                for n in range(0, HD, 256):
                    rhs = jnp.concatenate([x_term(u, _RHS_AS_LHS[i])[:, n:n + 256] for u in units], axis=0)
                    p = _dot(_wide(ps_v.at[i], slice(m, m + MT)), rhs)
                    if first:
                        n_v[i, m:m + MT, n:n + 256] = p
                    else:
                        n_v[i, m:m + MT, n:n + 256] += p

    x_cp(0).start()
    wk_cp(0, 0).start()
    wk_cp(1, 1).start()
    r16 = lax.broadcasted_iota(jnp.int32, (16, D), 0)
    wr = wr_ref[...].astype(F32).reshape(1, D)
    gw = gw_ref[...].astype(F32).reshape(1, D)
    rg_v[...] = jnp.where(r16 == 0, wr, jnp.where(r16 == 1, gw, 0.0)).astype(BF16)
    x_cp(0).wait()
    wk_cp(0, 0).wait()
    wk_cp(1, 1).wait()
    wk_cp(0, 1).start()
    wk_cp(1, 0).start()
    w11, w22 = wk_v[0, 0].T, wk_v[1, 1].T
    put_w_terms((1, 4, 0), [w11, None, None, w22])
    full = slice(0, HD)
    early = []
    for u in range(UC):
        route(u)
        make_x_terms(u)
        early.append({i: proj_term(u, i, full) for i in (1, 4, 0)})
    wk_cp(0, 1).wait()
    wk_cp(1, 0).wait()
    for c in range(1, NC):
        x_cp(c).start()
    put_w_terms((2, 3, 5, 6), [w11, wk_v[0, 1].T, wk_v[1, 0].T, w22])
    for u in range(UC):
        prods = dict(early[u])
        prods.update({i: proj_term(u, i, full) for i in (3, 6, 2, 5)})
        k_finish(u, full, prods, u == 0)
    for cp in (wq_cp, wv_cp, wo_cp):
        cp.start()
    for i in range(NC):
        for cp in f_cps(i):
            cp.start()
    t_part(range(UC), True)
    for c in range(1, NC):
        x_cp(c).wait()

    def p1(c, carry):
        units = [c * UC + t for t in range(UC)]
        for t, u in enumerate(units):
            make_x_terms(u)
            for m in range(0, HD, MQ):
                rows = slice(m, m + MQ)
                k_finish(t, rows, {i: proj_term(u, i, rows) for i in (2, 3, 0, 4, 6, 1, 5)}, False)
            route(u)
        t_part(units, False)
        return carry

    lax.fori_loop(1, NC, p1, 0)

    wq_cp.wait()
    wv_cp.wait()
    wo_cp.wait()
    for i in range(NC):
        for cp in f_cps(i):
            cp.wait()
    r = r_v[:, 0:1, :]
    tok = (lax.broadcasted_iota(jnp.int32, r.shape, 0) * UH
           + lax.broadcasted_iota(jnp.int32, r.shape, 2))
    best = jnp.max(jnp.max(jnp.where(r != r, -jnp.inf, r), axis=0), axis=1, keepdims=True)
    bidx = jnp.min(jnp.min(jnp.where(r == best, tok, S), axis=0), axis=1, keepdims=True)
    idx = jnp.where(bidx == S, 0, bidx)[0, 0]
    rsel = jnp.where(bidx == S, jnp.nan, best)
    base = pl.multiple_of((idx // 16) * 16, 16)
    sel = lax.broadcasted_iota(jnp.int32, (16, 1), 0) == idx - base
    xsel = jnp.sum(jnp.where(sel, x_v[pl.ds(base, 16), :].astype(F32), 0.0), axis=0, keepdims=True)
    xsel_v[...] = jnp.broadcast_to(xsel, (8, D))
    y_v[...] = jnp.zeros_like(y_v)

    put_w_terms(range(7), [wq_v[i * HD:(i + 1) * HD, j * HD:(j + 1) * HD].T for i in (0, 1) for j in (0, 1)])
    z_v[...] = jnp.broadcast_to(jnp.sum(z_v[...], axis=1, keepdims=True), z_v.shape)
    same_head = (lax.broadcasted_iota(jnp.int32, (128, 128), 0) // DH
                 == lax.broadcasted_iota(jnp.int32, (128, 128), 1) // DH)
    for j in range(0, HD, 128):
        t11, t12, t21, t22 = _combine([n_v[i, j:j + 128, :] for i in range(7)])
        m = []
        for o, t in ((j, (t11, t12)), (HD + j, (t21, t22))):
            kv = _dot(jnp.concatenate(t, axis=1).astype(BF16), wv_v[:, o:o + 128])
            kv = jnp.where(same_head, kv, 0.0).astype(BF16)
            m.append(_dot(kv, wo_v[o:o + 128, :]))
        for i, t in enumerate(_rhs_terms(m[0][:, :HD], m[0][:, HD:], m[1][:, :HD], m[1][:, HD:])):
            _put_wide(ms_v.at[i], slice(j, j + 128), t.astype(BF16))

    def ffn_steps(c):
        st = {}

        def proj(key, w_v, n, k):
            def step():
                p = _dot(xsel_v[:, k:k + HD], w_v[c, k:k + HD, n:n + 128])
                st[key, n] = p if k == 0 else st[key, n] + p
            return step

        def down(n, k):
            def step():
                if k == 0:
                    g = st['g', n]
                    st['h', n] = (g * _sigmoid(g) * st['u', n]).astype(BF16).astype(F32)
                y_v[:, k:k + HD] += _dot(st['h', n], wd_v[c, n:n + 128, k:k + HD])
            return step

        tiles = range(0, FC, 128)
        return ([proj(key, w_v, n, k) for n in tiles for key, w_v in (('g', wg_v), ('u', wu_v)) for k in (0, HD)]
                + [down(n, k) for n in tiles for k in (0, HD)])

    def mix(rows, cols, a, y=None):
        g = jnp.tile(g_v[rows, :], (1, a.shape[1] // 128))
        b = x_v[rows, cols].astype(F32)
        upd = b * 0.0 if y is None else b * 0.0 + y
        out_v[rows, cols] = (g * a + (1.0 - g) * (b + upd)).astype(BF16)

    def p2(c, carry):
        steps = ffn_steps(c) if CFG['FFN'] else []

        def with_ffn(p):
            if steps:
                steps.pop(0)()
            return p

        units = [(idx // U + 1 + c * UC + t) % NU for t in range(UC)]
        for t, u in enumerate(units):
            for m in range(0, HD, MQ):
                rows = slice(m, m + MQ)
                q = _combine({i: with_ffn(proj_term(u, i, rows)) for i in (2, 3, 0, 4, 6, 1, 5)})
                pqn = []
                for qij, o in zip(q, (m, HD + m, m, HD + m)):
                    pq = _phi(qij).reshape(MQ // DH, DH, UH)
                    den = jnp.sum(pq * z_v[o:o + MQ, :].reshape(MQ // DH, DH, UH), axis=1, keepdims=True) + 1e-6
                    pqn.append((pq * (1.0 / den)).reshape(MQ, UH))
                for i, p in enumerate(_lhs_terms(*pqn)):
                    _put_wide(rs_v.at[t, i, m // 128:(m + MQ) // 128], slice(None), p.T.astype(BF16))
        for t, u in enumerate(units):
            for n in range(0, HD, 128):
                a = _combine({i: with_ffn(_dot(_wide(rs_v.at[t, i]), ms_v[i, n // 128]))
                              for i in (0, 3, 4, 6, 2, 1, 5)})
                for aij, (i, j) in zip(a, ((0, 0), (0, 1), (1, 0), (1, 1))):
                    cols = slice(j * HD + n, j * HD + n + 128)
                    if t == UC - 1:
                        a_v[i * UH:(i + 1) * UH, cols] = aij
                    mix(pl.ds(pl.multiple_of(u * U + i * UH, UH), UH), cols, aij)
            if t < UC - 1:
                o_cp(u).start()
            else:
                pl.when(c < NC - 1)(o_cp(u).start)
        assert not steps
        return carry

    lax.fori_loop(0, NC, p2, 0)

    y = y_v[:1, :] * _sigmoid(rsel)
    mix(pl.ds(base, 16), slice(None), a_v[pl.ds(pl.multiple_of(base % U, 16), 16), :], jnp.where(sel, y, 0.0))
    o_cp(idx // U).start()
    for u in range(NU):
        o_cp(u).wait()


@jax.jit
def pallas_gated_mix__linear_attn_block__moe_arch_mod__prompt_kernel(
    A_x, A_wqkv, A_wo, B_x, B_w_r, B_w_gate, B_w_up, B_w_down, gate_w,
):
    del B_x
    hbm = pl.BlockSpec(memory_space=pl.ANY)
    vmem = pl.BlockSpec(memory_space=pltpu.VMEM)
    out = pl.pallas_call(
        _body,
        out_shape=jax.ShapeDtypeStruct((S, D), BF16),
        in_specs=[hbm, hbm, hbm, vmem, hbm, hbm, hbm, vmem],
        out_specs=hbm,
        scratch_shapes=[
            pltpu.VMEM((S, D), BF16),
            pltpu.VMEM((2, 2, HD, HD), BF16),
            pltpu.VMEM((D, D), BF16),
            pltpu.VMEM((D, D), BF16),
            pltpu.VMEM((D, D), BF16),
            pltpu.VMEM((NC, D, FC), BF16),
            pltpu.VMEM((NC, D, FC), BF16),
            pltpu.VMEM((NC, FC, D), BF16),
            pltpu.VMEM((5, S // 2, HD), BF16),
            pltpu.VMEM((7, HD // 128, HD, 128), BF16),
            pltpu.VMEM((7, UC, HD, UH), BF16),
            pltpu.VMEM((7, HD, HD), F32),
            pltpu.VMEM((D, 128), F32),
            pltpu.VMEM((7, HD // 128, HD, 128), BF16),
            pltpu.VMEM((UC, 7, HD // 128, UH, 128), BF16),
            pltpu.VMEM((16, D), BF16),
            pltpu.VMEM((S // UH, 8, UH), F32),
            pltpu.VMEM((S, 128), F32),
            pltpu.VMEM((U, D), F32),
            pltpu.VMEM((8, D), F32),
            pltpu.VMEM((8, D), F32),
            pltpu.VMEM((S, D), BF16),
            pltpu.SemaphoreType.DMA((NC,)),
            pltpu.SemaphoreType.DMA((7,)),
            pltpu.SemaphoreType.DMA((3, NC)),
            pltpu.SemaphoreType.DMA((NU,)),
        ],
        compiler_params=pltpu.CompilerParams(vmem_limit_bytes=100 * 1024 * 1024),
    )(A_x.reshape(S, D), A_wqkv, A_wo, B_w_r, B_w_gate, B_w_up, B_w_down, gate_w)
    return out.reshape(1, S, D)
```

```python
import jax
import jax.numpy as jnp
from jax import lax
import jax.experimental.pallas as pl
import jax.experimental.pallas.tpu as pltpu

CFG = dict(FFN=1, MQ=512, MT=512)

S, D, F, DH = 2048, 1024, 3584, 32
HD = D // 2
U = 256
UH = U // 2
NU = S // U
UC = 2
NC = NU // UC
FC = F // NC
F32, BF16, U32 = jnp.float32, jnp.bfloat16, jnp.uint32
NN = (((1,), (0,)), ((), ()))
NT = (((1,), (1,)), ((), ()))


def _dot(a, b, dims=NN):
    return lax.dot_general(a, b, dims, preferred_element_type=F32)


def _phi(t):
    return jnp.where(t > 0, t + 1.0, jnp.exp(t)) + 1e-6


def _sigmoid(t):
    return 1.0 / (1.0 + jnp.exp(-t))


def _lhs_terms(a11, a12, a21, a22):
    return [a11 + a22, a21 + a22, a11, a22, a11 + a12, a21 - a11, a12 - a22]


def _rhs_terms(b11, b12, b21, b22):
    return [b11 + b22, b11, b12 - b22, b21 - b11, b22, b11 + b12, b21 + b22]


def _combine(p):
    return p[0] + p[3] - p[4] + p[6], p[2] + p[4], p[1] + p[3], p[0] - p[1] + p[2] + p[5]


_RHS_AS_LHS = (0, 2, 6, 5, 3, 4, 1)


def _as_matrix(words):
    return pltpu.bitcast(words, BF16)


def _even_odd(mat):
    words = pltpu.bitcast(mat, U32)
    return [pltpu.unpack_elementwise(words, index=i, packed_dtype=BF16, unpacked_dtype=F32) for i in (0, 1)]


def _words(even, odd):
    return pltpu.bitcast(pltpu.pack_elementwise([even, odd], packed_dtype=BF16), U32)


def _words_riffled(v):
    return jnp.concatenate([_words(v[r:r + 64], v[r + 64:r + 128]) for r in range(0, v.shape[0], 128)], axis=0)


def _half(rows):
    return slice(rows.start // 2, rows.stop // 2)


def _body(x_hbm, wqkv_hbm, wo_hbm, wr_ref, wg_hbm, wu_hbm, wd_hbm, gw_ref, out_hbm,
          x_v, wk_v, wq_v, wv_v, wo_v, wg_v, wu_v, wd_v,
          xs_v, ws_v, ps_v, n_v, z_v, ms_v, rs_v, rg_v, r_v, g_v, a_v, xsel_v, y_v, out_v,
          sem_x, sem_w, sem_f, sem_o):
    MQ, MT = CFG['MQ'], CFG['MT']

    def x_cp(c):
        rows = pl.ds(c * UC * U, UC * U)
        return pltpu.make_async_copy(x_hbm.at[rows], x_v.at[rows], sem_x.at[c])

    def wk_cp(i, j):
        return pltpu.make_async_copy(wqkv_hbm.at[pl.ds(i * HD, HD), pl.ds(D + j * HD, HD)],
                                     wk_v.at[i, j], sem_w.at[2 * i + j])

    wq_cp = pltpu.make_async_copy(wqkv_hbm.at[:, pl.ds(0, D)], wq_v, sem_w.at[4])
    wv_cp = pltpu.make_async_copy(wqkv_hbm.at[:, pl.ds(2 * D, D)], wv_v, sem_w.at[5])
    wo_cp = pltpu.make_async_copy(wo_hbm, wo_v, sem_w.at[6])

    def f_cps(i):
        hid = pl.ds(pl.multiple_of(i * FC, 128), FC)
        return (pltpu.make_async_copy(wg_hbm.at[:, hid], wg_v.at[i], sem_f.at[0, i]),
                pltpu.make_async_copy(wu_hbm.at[:, hid], wu_v.at[i], sem_f.at[1, i]),
                pltpu.make_async_copy(wd_hbm.at[hid], wd_v.at[i], sem_f.at[2, i]))

    def o_cp(u):
        rows = pl.ds(pl.multiple_of(u * U, U), U)
        return pltpu.make_async_copy(out_v.at[rows], out_hbm.at[rows], sem_o.at[u])

    def x_quadrant(u, i, j):
        return x_v[pl.ds(pl.multiple_of(u * U + i * UH, UH), UH), j * HD:(j + 1) * HD]

    def make_x_terms(u):
        quads = [x_quadrant(u, i, j) for i in (0, 1) for j in (0, 1)]
        even, odd = zip(*[_even_odd(q) for q in quads])
        for i, (e, o) in enumerate(zip(_lhs_terms(*even), _lhs_terms(*odd))):
            xs_v[i, u] = pltpu.bitcast(quads[3 * (i - 2)], U32) if i in (2, 3) else _words(e, o)

    def x_term(u, i):
        return _as_matrix(xs_v[i, u])

    def put_w_terms(which, wt):
        f = [None if w is None else _even_odd(w) for w in wt]
        for i in which:
            if i in (1, 4):
                ws_v[i] = pltpu.bitcast(wt[0 if i == 1 else 3], U32)
            else:
                a, b, sign = {0: (0, 3, 1), 2: (1, 3, -1), 3: (2, 0, -1), 5: (0, 1, 1), 6: (2, 3, 1)}[i]
                ws_v[i] = _words(*[fa + fb if sign > 0 else fa - fb for fa, fb in zip(f[a], f[b])])

    def proj_term(u, i, rows):
        return _dot(_as_matrix(ws_v[i, _half(rows), :]), x_term(u, i), NT)

    def route(u):
        for h in range(2):
            o = pl.multiple_of(u * U + h * UH, UH)
            rg = _dot(rg_v[...], x_v[pl.ds(o, UH), :], NT)
            r_v[2 * u + h] = rg[:8].astype(BF16).astype(F32)
            g_v[pl.ds(o, UH), :] = jnp.broadcast_to(_sigmoid(rg[1:2]), (UH, UH)).T

    def k_finish(t, rows, prods, first):
        k11, k12, k21, k22 = [_phi(k) for k in _combine(prods)]
        lo, hi = rows, slice(HD + rows.start, HD + rows.stop)
        if first:
            z_v[lo, :] = k11 + k21
            z_v[hi, :] = k12 + k22
        else:
            z_v[lo, :] += k11 + k21
            z_v[hi, :] += k12 + k22
        for i, p in enumerate(_lhs_terms(k11, k21, k12, k22)):
            ps_v[i, _half(rows), t * UH:(t + 1) * UH] = _words_riffled(p)

    def t_part(units, first):
        for i in (1, 4, 0, 2, 3, 5, 6):
            for m in range(0, HD, MT):
                for n in range(0, HD, 256):
                    rhs = jnp.concatenate([_as_matrix(xs_v[_RHS_AS_LHS[i], u, :, n:n + 256]) for u in units], axis=0)
                    p = _dot(_as_matrix(ps_v[i, m // 2:(m + MT) // 2, :]), rhs)
                    for k in (0, 1):
                        if first:
                            n_v[i, n // 128 + k, m:m + MT, :] = p[:, k * 128:(k + 1) * 128]
                        else:
                            n_v[i, n // 128 + k, m:m + MT, :] += p[:, k * 128:(k + 1) * 128]

    x_cp(0).start()
    wk_cp(0, 0).start()
    wk_cp(1, 1).start()
    r16 = lax.broadcasted_iota(jnp.int32, (16, D), 0)
    wr = wr_ref[...].astype(F32).reshape(1, D)
    gw = gw_ref[...].astype(F32).reshape(1, D)
    rg_v[...] = jnp.where(r16 == 0, wr, jnp.where(r16 == 1, gw, 0.0)).astype(BF16)
    x_cp(0).wait()
    wk_cp(0, 0).wait()
    wk_cp(1, 1).wait()
    wk_cp(0, 1).start()
    wk_cp(1, 0).start()
    w11, w22 = wk_v[0, 0].T, wk_v[1, 1].T
    put_w_terms((1, 4, 0), [w11, None, None, w22])
    full = slice(0, HD)
    early = []
    for u in range(UC):
        route(u)
        make_x_terms(u)
        early.append({i: proj_term(u, i, full) for i in (1, 4, 0)})
    wk_cp(0, 1).wait()
    wk_cp(1, 0).wait()
    for c in range(1, NC):
        x_cp(c).start()
    put_w_terms((2, 3, 5, 6), [w11, wk_v[0, 1].T, wk_v[1, 0].T, w22])
    for u in range(UC):
        prods = dict(early[u])
        prods.update({i: proj_term(u, i, full) for i in (3, 6, 2, 5)})
        k_finish(u, full, prods, u == 0)
    t_part(range(UC), True)
    for c in range(1, NC):
        x_cp(c).wait()
    for cp in (wq_cp, wv_cp, wo_cp) + f_cps(0):
        cp.start()

    def p1(c, carry):
        for cp in f_cps(c):
            cp.start()
        units = [c * UC + t for t in range(UC)]
        for t, u in enumerate(units):
            make_x_terms(u)
            for m in range(0, HD, MQ):
                rows = slice(m, m + MQ)
                k_finish(t, rows, {i: proj_term(u, i, rows) for i in (2, 3, 0, 4, 6, 1, 5)}, False)
            route(u)
        t_part(units, False)
        return carry

    lax.fori_loop(1, NC, p1, 0)

    wq_cp.wait()
    wv_cp.wait()
    wo_cp.wait()
    r = r_v[:, 0:1, :]
    tok = (lax.broadcasted_iota(jnp.int32, r.shape, 0) * UH
           + lax.broadcasted_iota(jnp.int32, r.shape, 2))
    best = jnp.max(jnp.max(jnp.where(r != r, -jnp.inf, r), axis=0), axis=1, keepdims=True)
    bidx = jnp.min(jnp.min(jnp.where(r == best, tok, S), axis=0), axis=1, keepdims=True)
    idx = jnp.where(bidx == S, 0, bidx)[0, 0]
    rsel = jnp.where(bidx == S, jnp.nan, best)
    base = pl.multiple_of((idx // 16) * 16, 16)
    sel = lax.broadcasted_iota(jnp.int32, (16, 1), 0) == idx - base
    xsel = jnp.sum(jnp.where(sel, x_v[pl.ds(base, 16), :].astype(F32), 0.0), axis=0, keepdims=True)
    xsel_v[...] = jnp.broadcast_to(xsel, (8, D))
    y_v[...] = jnp.zeros_like(y_v)

    put_w_terms(range(7), [wq_v[i * HD:(i + 1) * HD, j * HD:(j + 1) * HD].T for i in (0, 1) for j in (0, 1)])
    z_v[...] = jnp.broadcast_to(jnp.sum(z_v[...], axis=1, keepdims=True), z_v.shape)
    same_head = ((lax.broadcasted_iota(jnp.int32, (128, 128), 0) // 16) % 4
                 == lax.broadcasted_iota(jnp.int32, (128, 128), 1) // DH)
    for j in range(0, HD, 128):
        t11, t12, t21, t22 = zip(*[_combine([
            jnp.concatenate([n_v[i, n, pl.ds(j + h, 32, stride=4), :] for h in range(4)], axis=0)
            for i in range(7)]) for n in range(HD // 128)])
        m = []
        for o, t in ((j, t11 + t12), (HD + j, t21 + t22)):
            kv = _dot(jnp.concatenate(t, axis=1).astype(BF16), wv_v[:, o:o + 128])
            kv = jnp.where(same_head, kv, 0.0).astype(BF16)
            m.append(_dot(kv, wo_v[o:o + 128, :]))
        for i, t in enumerate(_rhs_terms(m[0][:, :HD], m[0][:, HD:], m[1][:, :HD], m[1][:, HD:])):
            ms_v[i, j // 2:j // 2 + 64, :] = _words(t[:64], t[64:])

    def ffn_steps(c):
        st = {}

        def proj(key, w_v, n, k):
            def step():
                p = _dot(xsel_v[:, k:k + HD], w_v[c, k:k + HD, n:n + 128])
                st[key, n] = p if k == 0 else st[key, n] + p
            return step

        def down(n, k):
            def step():
                if k == 0:
                    g = st['g', n]
                    st['h', n] = (g * _sigmoid(g) * st['u', n]).astype(BF16).astype(F32)
                y_v[:, k:k + HD] += _dot(st['h', n], wd_v[c, n:n + 128, k:k + HD])
            return step

        tiles = range(0, FC, 128)
        return ([proj(key, w_v, n, k) for n in tiles for key, w_v in (('g', wg_v), ('u', wu_v)) for k in (0, HD)]
                + [down(n, k) for n in tiles for k in (0, HD)])

    def mix(rows, cols, a, y=None):
        g = jnp.tile(g_v[rows, :], (1, a.shape[1] // 128))
        b = x_v[rows, cols].astype(F32)
        upd = b * 0.0 if y is None else b * 0.0 + y
        out_v[rows, cols] = (g * a + (1.0 - g) * (b + upd)).astype(BF16)

    def p2(c, carry):
        for cp in f_cps(c):
            cp.wait()
        steps = ffn_steps(c) if CFG['FFN'] else []

        def with_ffn(p):
            if steps:
                steps.pop(0)()
            return p

        units = [(idx // U + 1 + c * UC + t) % NU for t in range(UC)]
        for t, u in enumerate(units):
            for m in range(0, HD, MQ):
                rows = slice(m, m + MQ)
                q = _combine({i: with_ffn(proj_term(u, i, rows)) for i in (2, 3, 0, 4, 6, 1, 5)})
                pqn = []
                for qij, o in zip(q, (m, HD + m, m, HD + m)):
                    pq = _phi(qij).reshape(MQ // DH, DH, UH)
                    den = jnp.sum(pq * z_v[o:o + MQ, :].reshape(MQ // DH, DH, UH), axis=1, keepdims=True) + 1e-6
                    pqn.append((pq * (1.0 / den)).reshape(MQ, UH))
                for i, p in enumerate(_lhs_terms(*pqn)):
                    rs_v[t, i, :, rows] = _words_riffled(p.T)
        for t, u in enumerate(units):
            for n in range(0, HD, 128):
                a = _combine({i: with_ffn(_dot(_as_matrix(rs_v[t, i]), _as_matrix(ms_v[i, :, n:n + 128])))
                              for i in (0, 3, 4, 6, 2, 1, 5)})
                for aij, (i, j) in zip(a, ((0, 0), (0, 1), (1, 0), (1, 1))):
                    cols = slice(j * HD + n, j * HD + n + 128)
                    a_v[2 * i + j, n // 128] = aij
                    aij = jnp.concatenate([a_v[2 * i + j, n // 128, pl.ds(h, 64, stride=2), :] for h in (0, 1)], axis=0)
                    mix(pl.ds(pl.multiple_of(u * U + i * UH, UH), UH), cols, aij)
            if t < UC - 1:
                o_cp(u).start()
            else:
                pl.when(c < NC - 1)(o_cp(u).start)
        assert not steps
        return carry

    lax.fori_loop(0, NC, p2, 0)

    y = y_v[:1, :] * _sigmoid(rsel)
    i, row = (base % U) // UH, 2 * (base % 64) + (base % UH) // 64
    a = jnp.concatenate([a_v[2 * i + j, n, pl.ds(row, 16, stride=2), :]
                         for j in (0, 1) for n in range(HD // 128)], axis=1)
    mix(pl.ds(base, 16), slice(None), a, jnp.where(sel, y, 0.0))
    o_cp(idx // U).start()
    for u in range(NU):
        o_cp(u).wait()


@jax.jit
def pallas_gated_mix__linear_attn_block__moe_arch_mod__prompt_kernel(
    A_x, A_wqkv, A_wo, B_x, B_w_r, B_w_gate, B_w_up, B_w_down, gate_w,
):
    del B_x
    hbm = pl.BlockSpec(memory_space=pl.ANY)
    vmem = pl.BlockSpec(memory_space=pltpu.VMEM)
    out = pl.pallas_call(
        _body,
        out_shape=jax.ShapeDtypeStruct((S, D), BF16),
        in_specs=[hbm, hbm, hbm, vmem, hbm, hbm, hbm, vmem],
        out_specs=hbm,
        scratch_shapes=[
            pltpu.VMEM((S, D), BF16),
            pltpu.VMEM((2, 2, HD, HD), BF16),
            pltpu.VMEM((D, D), BF16),
            pltpu.VMEM((D, D), BF16),
            pltpu.VMEM((D, D), BF16),
            pltpu.VMEM((NC, D, FC), BF16),
            pltpu.VMEM((NC, D, FC), BF16),
            pltpu.VMEM((NC, FC, D), BF16),
            pltpu.VMEM((7, NU, UH // 2, HD), U32),
            pltpu.VMEM((7, HD // 2, HD), U32),
            pltpu.VMEM((7, HD // 2, UC * UH), U32),
            pltpu.VMEM((7, HD // 128, HD, 128), F32),
            pltpu.VMEM((D, 128), F32),
            pltpu.VMEM((7, HD // 2, HD), U32),
            pltpu.VMEM((UC, 7, UH // 2, HD), U32),
            pltpu.VMEM((16, D), BF16),
            pltpu.VMEM((S // UH, 8, UH), F32),
            pltpu.VMEM((S, 128), F32),
            pltpu.VMEM((4, HD // 128, UH, 128), F32),
            pltpu.VMEM((8, D), F32),
            pltpu.VMEM((8, D), F32),
            pltpu.VMEM((S, D), BF16),
            pltpu.SemaphoreType.DMA((NC,)),
            pltpu.SemaphoreType.DMA((7,)),
            pltpu.SemaphoreType.DMA((3, NC)),
            pltpu.SemaphoreType.DMA((NU,)),
        ],
        compiler_params=pltpu.CompilerParams(vmem_limit_bytes=100 * 1024 * 1024),
    )(A_x.reshape(S, D), A_wqkv, A_wo, B_w_r, B_w_gate, B_w_up, B_w_down, gate_w)
    return out.reshape(1, S, D)
```

```python
import jax
import jax.numpy as jnp
from jax import lax
import jax.experimental.pallas as pl
import jax.experimental.pallas.tpu as pltpu

CFG = dict(FFN=1, MQ=512, MT=256)

S, D, F, DH = 2048, 1024, 3584, 32
HD = D // 2
U = 256
UH = U // 2
NU = S // U
UC = 2
NC = NU // UC
FC = F // NC
F32, BF16, U32 = jnp.float32, jnp.bfloat16, jnp.uint32
NN = (((1,), (0,)), ((), ()))
NT = (((1,), (1,)), ((), ()))


def _dot(a, b, dims=NN):
    return lax.dot_general(a, b, dims, preferred_element_type=F32)


def _phi(t):
    return jnp.where(t > 0, t + 1.0, jnp.exp(t)) + 1e-6


def _sigmoid(t):
    return 1.0 / (1.0 + jnp.exp(-t))


def _lhs_terms(a11, a12, a21, a22):
    return [a11 + a22, a21 + a22, a11, a22, a11 + a12, a21 - a11, a12 - a22]


def _rhs_terms(b11, b12, b21, b22):
    return [b11 + b22, b11, b12 - b22, b21 - b11, b22, b11 + b12, b21 + b22]


def _combine(p):
    return p[0] + p[3] - p[4] + p[6], p[2] + p[4], p[1] + p[3], p[0] - p[1] + p[2] + p[5]


_RHS_AS_LHS = (0, 2, 6, 5, 3, 4, 1)


def _as_matrix(words):
    return pltpu.bitcast(words, BF16)


def _even_odd(mat):
    words = pltpu.bitcast(mat, U32)
    return [pltpu.unpack_elementwise(words, index=i, packed_dtype=BF16, unpacked_dtype=F32) for i in (0, 1)]


def _words(even, odd):
    return pltpu.bitcast(pltpu.pack_elementwise([even, odd], packed_dtype=BF16), U32)


def _words_riffled(v):
    return jnp.concatenate([_words(v[r:r + 64], v[r + 64:r + 128]) for r in range(0, v.shape[0], 128)], axis=0)


def _half(rows):
    return slice(rows.start // 2, rows.stop // 2)


def _body(x_hbm, wqkv_hbm, wo_hbm, wr_ref, wg_hbm, wu_hbm, wd_hbm, gw_ref, out_hbm,
          x_v, wk_v, wq_v, wv_v, wo_v, wg_v, wu_v, wd_v,
          xs_v, ws_v, ps_v, t_v, z_v, ms_v, rs_v, rg_v, r_v, g_v, a_v, xsel_v, y_v, out_v,
          sem_x, sem_w, sem_f, sem_o):
    MQ, MT = CFG['MQ'], CFG['MT']

    def x_cp(c):
        rows = pl.ds(c * UC * U, UC * U)
        return pltpu.make_async_copy(x_hbm.at[rows], x_v.at[rows], sem_x.at[c])

    def wk_cp(i, j):
        return pltpu.make_async_copy(wqkv_hbm.at[pl.ds(i * HD, HD), pl.ds(D + j * HD, HD)],
                                     wk_v.at[i, j], sem_w.at[2 * i + j])

    wq_cp = pltpu.make_async_copy(wqkv_hbm.at[:, pl.ds(0, D)], wq_v, sem_w.at[4])
    wv_cp = pltpu.make_async_copy(wqkv_hbm.at[:, pl.ds(2 * D, D)], wv_v, sem_w.at[5])
    wo_cp = pltpu.make_async_copy(wo_hbm, wo_v, sem_w.at[6])

    def f_cps(i):
        hid = pl.ds(pl.multiple_of(i * FC, 128), FC)
        return (pltpu.make_async_copy(wg_hbm.at[:, hid], wg_v.at[i], sem_f.at[0, i]),
                pltpu.make_async_copy(wu_hbm.at[:, hid], wu_v.at[i], sem_f.at[1, i]),
                pltpu.make_async_copy(wd_hbm.at[hid], wd_v.at[i], sem_f.at[2, i]))

    def o_cp(u):
        rows = pl.ds(pl.multiple_of(u * U, U), U)
        return pltpu.make_async_copy(out_v.at[rows], out_hbm.at[rows], sem_o.at[u])

    def make_x_terms(u):
        for n in range(0, HD, 128):
            quads = [x_v[pl.ds(pl.multiple_of(u * U + i * UH, UH), UH), j * HD + n:j * HD + n + 128]
                     for i in (0, 1) for j in (0, 1)]
            even, odd = zip(*[_even_odd(q) for q in quads])
            for i, (e, o) in enumerate(zip(_lhs_terms(*even), _lhs_terms(*odd))):
                xs_v[i, u, :, n:n + 128] = pltpu.bitcast(quads[3 * (i - 2)], U32) if i in (2, 3) else _words(e, o)

    def x_term(u, i):
        return _as_matrix(xs_v[i, u])

    def put_w_terms(which, quadrant):
        pairs = {0: (0, 3, 1), 2: (1, 3, -1), 3: (2, 0, -1), 5: (0, 1, 1), 6: (2, 3, 1)}
        for r in range(0, HD, 128):
            for n in range(0, HD, 128):
                wt = [quadrant(a)[n:n + 128, r:r + 128].T for a in range(4)]
                f = [_even_odd(w) for w in wt]
                for i in which:
                    if i in pairs:
                        a, b, sign = pairs[i]
                        t = _words(*[fa + fb if sign > 0 else fa - fb for fa, fb in zip(f[a], f[b])])
                    else:
                        t = pltpu.bitcast(wt[0 if i == 1 else 3], U32)
                    ws_v[i, r // 2:r // 2 + 64, n:n + 128] = t

    def proj_term(u, i, rows):
        return _dot(_as_matrix(ws_v[i, _half(rows), :]), x_term(u, i), NT)

    def route(u):
        for h in range(2):
            o = pl.multiple_of(u * U + h * UH, UH)
            rg = _dot(rg_v[...], x_v[pl.ds(o, UH), :], NT)
            r_v[2 * u + h] = rg[:8].astype(BF16).astype(F32)
            g_v[pl.ds(o, UH), :] = jnp.broadcast_to(_sigmoid(rg[1:2]), (UH, UH)).T

    def k_finish(t, rows, prods, first):
        k11, k12, k21, k22 = [_phi(k) for k in _combine(prods)]
        lo, hi = rows, slice(HD + rows.start, HD + rows.stop)
        if first:
            z_v[lo, :] = k11 + k21
            z_v[hi, :] = k12 + k22
        else:
            z_v[lo, :] += k11 + k21
            z_v[hi, :] += k12 + k22
        for i, p in enumerate(_lhs_terms(k11, k21, k12, k22)):
            ps_v[i, _half(rows), t * UH:(t + 1) * UH] = _words_riffled(p)

    def t_part(units, first):
        for m in range(0, HD, MT):
            for n in range(0, HD, 256):
                prods = {}
                for i in (0, 3, 4, 6, 2, 1, 5):
                    rhs = jnp.concatenate([xs_v[_RHS_AS_LHS[i], u, :, n:n + 256] for u in units], axis=0)
                    prods[i] = _dot(_as_matrix(ps_v[i, m // 2:(m + MT) // 2, :]), _as_matrix(rhs))
                for t, (i, j) in zip(_combine(prods), ((0, 0), (0, 1), (1, 0), (1, 1))):
                    rows = slice(i * HD + m, i * HD + m + MT)
                    for k in (0, 128):
                        if first:
                            t_v[(j * HD + n + k) // 128, rows, :] = t[:, k:k + 128]
                        else:
                            t_v[(j * HD + n + k) // 128, rows, :] += t[:, k:k + 128]

    x_cp(0).start()
    wk_cp(0, 0).start()
    wk_cp(1, 1).start()
    r16 = lax.broadcasted_iota(jnp.int32, (16, D), 0)
    wr = wr_ref[...].astype(F32).reshape(1, D)
    gw = gw_ref[...].astype(F32).reshape(1, D)
    rg_v[...] = jnp.where(r16 == 0, wr, jnp.where(r16 == 1, gw, 0.0)).astype(BF16)
    x_cp(0).wait()
    wk_cp(0, 0).wait()
    wk_cp(1, 1).wait()
    wk_cp(0, 1).start()
    wk_cp(1, 0).start()
    put_w_terms((1, 4, 0), lambda a: wk_v.at[a // 2, a // 2])
    full = slice(0, HD)
    early = []
    for u in range(UC):
        route(u)
        make_x_terms(u)
        early.append({i: proj_term(u, i, full) for i in (1, 4, 0)})
    wk_cp(0, 1).wait()
    wk_cp(1, 0).wait()
    for c in range(1, NC):
        x_cp(c).start()
    put_w_terms((2, 3, 5, 6), lambda a: wk_v.at[a // 2, a % 2])
    for u in range(UC):
        prods = dict(early[u])
        prods.update({i: proj_term(u, i, full) for i in (3, 6, 2, 5)})
        k_finish(u, full, prods, u == 0)
    t_part(range(UC), True)
    for c in range(1, NC):
        x_cp(c).wait()
    for cp in (wq_cp, wv_cp, wo_cp) + f_cps(0):
        cp.start()

    def p1(c, carry):
        for cp in f_cps(c):
            cp.start()
        units = [c * UC + t for t in range(UC)]
        for t, u in enumerate(units):
            make_x_terms(u)
            for m in range(0, HD, MQ):
                rows = slice(m, m + MQ)
                k_finish(t, rows, {i: proj_term(u, i, rows) for i in (2, 3, 0, 4, 6, 1, 5)}, False)
            route(u)
        t_part(units, False)
        return carry

    lax.fori_loop(1, NC, p1, 0)

    wq_cp.wait()
    wv_cp.wait()
    wo_cp.wait()
    r = r_v[:, 0:1, :]
    tok = (lax.broadcasted_iota(jnp.int32, r.shape, 0) * UH
           + lax.broadcasted_iota(jnp.int32, r.shape, 2))
    best = jnp.max(jnp.max(jnp.where(r != r, -jnp.inf, r), axis=0), axis=1, keepdims=True)
    bidx = jnp.min(jnp.min(jnp.where(r == best, tok, S), axis=0), axis=1, keepdims=True)
    idx = jnp.where(bidx == S, 0, bidx)[0, 0]
    rsel = jnp.where(bidx == S, jnp.nan, best)
    base = pl.multiple_of((idx // 16) * 16, 16)
    sel = lax.broadcasted_iota(jnp.int32, (16, 1), 0) == idx - base
    xsel = jnp.sum(jnp.where(sel, x_v[pl.ds(base, 16), :].astype(F32), 0.0), axis=0, keepdims=True)
    xsel_v[...] = jnp.broadcast_to(xsel, (8, D))
    y_v[...] = jnp.zeros_like(y_v)

    put_w_terms(range(7), lambda a: wq_v.at[pl.ds(a // 2 * HD, HD), pl.ds(a % 2 * HD, HD)])
    z_v[...] = jnp.broadcast_to(jnp.sum(z_v[...], axis=1, keepdims=True), z_v.shape)
    same_head = ((lax.broadcasted_iota(jnp.int32, (128, 128), 0) // 16) % 4
                 == lax.broadcasted_iota(jnp.int32, (128, 128), 1) // DH)
    kvs = {}
    for o in range(0, D, 128):
        t = jnp.concatenate([
            jnp.concatenate([t_v[n, pl.ds(o + h, 32, stride=4), :] for h in range(4)], axis=0)
            for n in range(D // 128)], axis=1)
        kvs[o] = jnp.where(same_head, _dot(t.astype(BF16), wv_v[:, o:o + 128]), 0.0).astype(BF16)
    for j in range(0, HD, 128):
        for n in range(0, HD, 256):
            m = [_dot(kvs[o], wo_v[o:o + 128, h + n:h + n + 256]) for o in (j, HD + j) for h in (0, HD)]
            for i, t in enumerate(_rhs_terms(*m)):
                ms_v[i, j // 2:j // 2 + 64, n:n + 256] = _words(t[:64], t[64:])

    def ffn_steps(c):
        st = {}

        def proj(key, w_v, n, k):
            def step():
                p = _dot(xsel_v[:, k:k + HD], w_v[c, k:k + HD, n:n + 128])
                st[key, n] = p if k == 0 else st[key, n] + p
            return step

        def down(n, k):
            def step():
                if k == 0:
                    g = st['g', n]
                    st['h', n] = (g * _sigmoid(g) * st['u', n]).astype(BF16).astype(F32)
                y_v[:, k:k + HD] += _dot(st['h', n], wd_v[c, n:n + 128, k:k + HD])
            return step

        tiles = range(0, FC, 128)
        return ([proj(key, w_v, n, k) for n in tiles for key, w_v in (('g', wg_v), ('u', wu_v)) for k in (0, HD)]
                + [down(n, k) for n in tiles for k in (0, HD)])

    def mix(rows, cols, a, y=None):
        g = jnp.tile(g_v[rows, :], (1, a.shape[1] // 128))
        b = x_v[rows, cols].astype(F32)
        upd = b * 0.0 if y is None else b * 0.0 + y
        out_v[rows, cols] = (g * a + (1.0 - g) * (b + upd)).astype(BF16)

    def p2(c, carry):
        for cp in f_cps(c):
            cp.wait()
        steps = ffn_steps(c) if CFG['FFN'] else []

        def with_ffn(p):
            if steps:
                steps.pop(0)()
            return p

        units = [(idx // U + 1 + c * UC + t) % NU for t in range(UC)]
        for t, u in enumerate(units):
            for m in range(0, HD, MQ):
                rows = slice(m, m + MQ)
                q = _combine({i: with_ffn(proj_term(u, i, rows)) for i in (2, 3, 0, 4, 6, 1, 5)})
                pqn = []
                for qij, o in zip(q, (m, HD + m, m, HD + m)):
                    pq = _phi(qij).reshape(MQ // DH, DH, UH)
                    den = jnp.sum(pq * z_v[o:o + MQ, :].reshape(MQ // DH, DH, UH), axis=1, keepdims=True) + 1e-6
                    pqn.append((pq * (1.0 / den)).reshape(MQ, UH))
                for i, p in enumerate(_lhs_terms(*pqn)):
                    rs_v[t, i, :, rows] = _words_riffled(p.T)
        for t, u in enumerate(units):
            for n in range(0, HD, 128):
                a = _combine({i: with_ffn(_dot(_as_matrix(rs_v[t, i]), _as_matrix(ms_v[i, :, n:n + 128])))
                              for i in (0, 3, 4, 6, 2, 1, 5)})
                for aij, (i, j) in zip(a, ((0, 0), (0, 1), (1, 0), (1, 1))):
                    cols = slice(j * HD + n, j * HD + n + 128)
                    a_v[2 * i + j, n // 128] = aij
                    aij = jnp.concatenate([a_v[2 * i + j, n // 128, pl.ds(h, 64, stride=2), :] for h in (0, 1)], axis=0)
                    mix(pl.ds(pl.multiple_of(u * U + i * UH, UH), UH), cols, aij)
            if t < UC - 1:
                o_cp(u).start()
            else:
                pl.when(c < NC - 1)(o_cp(u).start)
        assert not steps
        return carry

    lax.fori_loop(0, NC, p2, 0)

    y = y_v[:1, :] * _sigmoid(rsel)
    i, row = (base % U) // UH, 2 * (base % 64) + (base % UH) // 64
    a = jnp.concatenate([a_v[2 * i + j, n, pl.ds(row, 16, stride=2), :]
                         for j in (0, 1) for n in range(HD // 128)], axis=1)
    mix(pl.ds(base, 16), slice(None), a, jnp.where(sel, y, 0.0))
    o_cp(idx // U).start()
    for u in range(NU):
        o_cp(u).wait()


@jax.jit
def pallas_gated_mix__linear_attn_block__moe_arch_mod__prompt_kernel(
    A_x, A_wqkv, A_wo, B_x, B_w_r, B_w_gate, B_w_up, B_w_down, gate_w,
):
    del B_x
    hbm = pl.BlockSpec(memory_space=pl.ANY)
    vmem = pl.BlockSpec(memory_space=pltpu.VMEM)
    out = pl.pallas_call(
        _body,
        out_shape=jax.ShapeDtypeStruct((S, D), BF16),
        in_specs=[hbm, hbm, hbm, vmem, hbm, hbm, hbm, vmem],
        out_specs=hbm,
        scratch_shapes=[
            pltpu.VMEM((S, D), BF16),
            pltpu.VMEM((2, 2, HD, HD), BF16),
            pltpu.VMEM((D, D), BF16),
            pltpu.VMEM((D, D), BF16),
            pltpu.VMEM((D, D), BF16),
            pltpu.VMEM((NC, D, FC), BF16),
            pltpu.VMEM((NC, D, FC), BF16),
            pltpu.VMEM((NC, FC, D), BF16),
            pltpu.VMEM((7, NU, UH // 2, HD), U32),
            pltpu.VMEM((7, HD // 2, HD), U32),
            pltpu.VMEM((7, HD // 2, UC * UH), U32),
            pltpu.VMEM((D // 128, D, 128), F32),
            pltpu.VMEM((D, 128), F32),
            pltpu.VMEM((7, HD // 2, HD), U32),
            pltpu.VMEM((UC, 7, UH // 2, HD), U32),
            pltpu.VMEM((16, D), BF16),
            pltpu.VMEM((S // UH, 8, UH), F32),
            pltpu.VMEM((S, 128), F32),
            pltpu.VMEM((4, HD // 128, UH, 128), F32),
            pltpu.VMEM((8, D), F32),
            pltpu.VMEM((8, D), F32),
            pltpu.VMEM((S, D), BF16),
            pltpu.SemaphoreType.DMA((NC,)),
            pltpu.SemaphoreType.DMA((7,)),
            pltpu.SemaphoreType.DMA((3, NC)),
            pltpu.SemaphoreType.DMA((NU,)),
        ],
        compiler_params=pltpu.CompilerParams(vmem_limit_bytes=100 * 1024 * 1024),
    )(A_x.reshape(S, D), A_wqkv, A_wo, B_w_r, B_w_gate, B_w_up, B_w_down, gate_w)
    return out.reshape(1, S, D)
```

```python
import jax
import jax.numpy as jnp
from jax import lax
import jax.experimental.pallas as pl
import jax.experimental.pallas.tpu as pltpu

CFG = dict(FFN=1, MQ=512, MT=256, NA=128)

S, D, F, DH = 2048, 1024, 3584, 32
HD = D // 2
U = 256
UH = U // 2
NU = S // U
UC = 2
NC = NU // UC
FC = F // NC
F32, BF16, U32 = jnp.float32, jnp.bfloat16, jnp.uint32
NN = (((1,), (0,)), ((), ()))
NT = (((1,), (1,)), ((), ()))


def _dot(a, b, dims=NN):
    return lax.dot_general(a, b, dims, preferred_element_type=F32)


def _phi(t):
    return jnp.where(t > 0, t + 1.0, jnp.exp(t)) + 1e-6


def _sigmoid(t):
    return 1.0 / (1.0 + jnp.exp(-t))


def _lhs_terms(a11, a12, a21, a22):
    return [a11 + a22, a21 + a22, a11, a22, a11 + a12, a21 - a11, a12 - a22]


def _rhs_terms(b11, b12, b21, b22):
    return [b11 + b22, b11, b12 - b22, b21 - b11, b22, b11 + b12, b21 + b22]


def _combine(p):
    return p[0] + p[3] - p[4] + p[6], p[2] + p[4], p[1] + p[3], p[0] - p[1] + p[2] + p[5]


_RHS_AS_LHS = (0, 2, 6, 5, 3, 4, 1)


def _as_matrix(words):
    return pltpu.bitcast(words, BF16)


def _even_odd(mat):
    words = pltpu.bitcast(mat, U32)
    return [pltpu.unpack_elementwise(words, index=i, packed_dtype=BF16, unpacked_dtype=F32) for i in (0, 1)]


def _words(even, odd):
    return pltpu.bitcast(pltpu.pack_elementwise([even, odd], packed_dtype=BF16), U32)


def _words_riffled(v):
    return jnp.concatenate([_words(v[r:r + 64], v[r + 64:r + 128]) for r in range(0, v.shape[0], 128)], axis=0)


def _half(rows):
    return slice(rows.start // 2, rows.stop // 2)


def _body(x_hbm, wqkv_hbm, wo_hbm, wr_ref, wg_hbm, wu_hbm, wd_hbm, gw_ref, out_hbm,
          x_v, wk_v, wq_v, wv_v, wo_v, wg_v, wu_v, wd_v,
          xs_v, ws_v, ps_v, t_v, z_v, ms_v, rs_v, rg_v, r_v, g_v, a_v, xsel_v, y_v, out_v,
          sem_x, sem_w, sem_f, sem_o):
    MQ, MT, NA = CFG['MQ'], CFG['MT'], CFG['NA']

    def x_cp(c):
        rows = pl.ds(c * UC * U, UC * U)
        return pltpu.make_async_copy(x_hbm.at[rows], x_v.at[rows], sem_x.at[c])

    def wk_cp(i, j):
        return pltpu.make_async_copy(wqkv_hbm.at[pl.ds(i * HD, HD), pl.ds(D + j * HD, HD)],
                                     wk_v.at[i, j], sem_w.at[2 * i + j])

    wq_cp = pltpu.make_async_copy(wqkv_hbm.at[:, pl.ds(0, D)], wq_v, sem_w.at[4])
    wv_cp = pltpu.make_async_copy(wqkv_hbm.at[:, pl.ds(2 * D, D)], wv_v, sem_w.at[5])
    wo_cp = pltpu.make_async_copy(wo_hbm, wo_v, sem_w.at[6])

    def f_cps(i):
        hid = pl.ds(pl.multiple_of(i * FC, 128), FC)
        return (pltpu.make_async_copy(wg_hbm.at[:, hid], wg_v.at[i], sem_f.at[0, i]),
                pltpu.make_async_copy(wu_hbm.at[:, hid], wu_v.at[i], sem_f.at[1, i]),
                pltpu.make_async_copy(wd_hbm.at[hid], wd_v.at[i], sem_f.at[2, i]))

    def o_cp(u):
        rows = pl.ds(pl.multiple_of(u * U, U), U)
        return pltpu.make_async_copy(out_v.at[rows], out_hbm.at[rows], sem_o.at[u])

    def make_x_terms(u):
        for n in range(0, HD, 128):
            quads = [x_v[pl.ds(pl.multiple_of(u * U + i * UH, UH), UH), j * HD + n:j * HD + n + 128]
                     for i in (0, 1) for j in (0, 1)]
            even, odd = zip(*[_even_odd(q) for q in quads])
            for i, (e, o) in enumerate(zip(_lhs_terms(*even), _lhs_terms(*odd))):
                xs_v[i, u, :, n:n + 128] = pltpu.bitcast(quads[3 * (i - 2)], U32) if i in (2, 3) else _words(e, o)

    def x_term(u, i):
        return _as_matrix(xs_v[i, u])

    def put_w_terms(which, quadrant):
        pairs = {0: (0, 3, 1), 2: (1, 3, -1), 3: (2, 0, -1), 5: (0, 1, 1), 6: (2, 3, 1)}
        for r in range(0, HD, 128):
            for n in range(0, HD, 128):
                wt = [quadrant(a)[n:n + 128, r:r + 128].T for a in range(4)]
                f = [_even_odd(w) for w in wt]
                for i in which:
                    if i in pairs:
                        a, b, sign = pairs[i]
                        t = _words(*[fa + fb if sign > 0 else fa - fb for fa, fb in zip(f[a], f[b])])
                    else:
                        t = pltpu.bitcast(wt[0 if i == 1 else 3], U32)
                    ws_v[i, r // 2:r // 2 + 64, n:n + 128] = t

    def proj_term(u, i, rows):
        return _dot(_as_matrix(ws_v[i, _half(rows), :]), x_term(u, i), NT)

    def route(u):
        for h in range(2):
            o = pl.multiple_of(u * U + h * UH, UH)
            rg = _dot(rg_v[...], x_v[pl.ds(o, UH), :], NT)
            r_v[2 * u + h] = rg[:8].astype(BF16).astype(F32)
            g_v[pl.ds(o, UH), :] = jnp.broadcast_to(_sigmoid(rg[1:2]), (UH, UH)).T

    def k_finish(t, rows, prods, first):
        k11, k12, k21, k22 = [_phi(k) for k in _combine(prods)]
        lo, hi = rows, slice(HD + rows.start, HD + rows.stop)
        if first:
            z_v[lo, :] = k11 + k21
            z_v[hi, :] = k12 + k22
        else:
            z_v[lo, :] += k11 + k21
            z_v[hi, :] += k12 + k22
        for i, p in enumerate(_lhs_terms(k11, k21, k12, k22)):
            ps_v[i, _half(rows), t * UH:(t + 1) * UH] = _words_riffled(p)

    def t_part(units, first):
        for m in range(0, HD, MT):
            for n in range(0, HD, 256):
                prods = {}
                for i in (0, 3, 4, 6, 2, 1, 5):
                    rhs = jnp.concatenate([xs_v[_RHS_AS_LHS[i], u, :, n:n + 256] for u in units], axis=0)
                    prods[i] = _dot(_as_matrix(ps_v[i, m // 2:(m + MT) // 2, :]), _as_matrix(rhs))
                for t, (i, j) in zip(_combine(prods), ((0, 0), (0, 1), (1, 0), (1, 1))):
                    rows = slice(i * HD + m, i * HD + m + MT)
                    for k in (0, 128):
                        if first:
                            t_v[(j * HD + n + k) // 128, rows, :] = t[:, k:k + 128]
                        else:
                            t_v[(j * HD + n + k) // 128, rows, :] += t[:, k:k + 128]

    x_cp(0).start()
    wk_cp(0, 0).start()
    wk_cp(1, 1).start()
    r16 = lax.broadcasted_iota(jnp.int32, (16, D), 0)
    wr = wr_ref[...].astype(F32).reshape(1, D)
    gw = gw_ref[...].astype(F32).reshape(1, D)
    rg_v[...] = jnp.where(r16 == 0, wr, jnp.where(r16 == 1, gw, 0.0)).astype(BF16)
    x_cp(0).wait()
    wk_cp(0, 0).wait()
    wk_cp(1, 1).wait()
    wk_cp(0, 1).start()
    wk_cp(1, 0).start()
    put_w_terms((1, 4, 0), lambda a: wk_v.at[a // 2, a // 2])
    full = slice(0, HD)
    early = []
    for u in range(UC):
        route(u)
        make_x_terms(u)
        early.append({i: proj_term(u, i, full) for i in (1, 4, 0)})
    wk_cp(0, 1).wait()
    wk_cp(1, 0).wait()
    for c in range(1, NC):
        x_cp(c).start()
    put_w_terms((2, 3, 5, 6), lambda a: wk_v.at[a // 2, a % 2])
    for u in range(UC):
        prods = dict(early[u])
        prods.update({i: proj_term(u, i, full) for i in (3, 6, 2, 5)})
        k_finish(u, full, prods, u == 0)
    t_part(range(UC), True)
    for c in range(1, NC):
        x_cp(c).wait()
    for cp in (wq_cp, wv_cp, wo_cp) + f_cps(0):
        cp.start()

    def p1(c, carry):
        for cp in f_cps(c):
            cp.start()
        units = [c * UC + t for t in range(UC)]
        for t, u in enumerate(units):
            make_x_terms(u)
            for m in range(0, HD, MQ):
                rows = slice(m, m + MQ)
                k_finish(t, rows, {i: proj_term(u, i, rows) for i in (2, 3, 0, 4, 6, 1, 5)}, False)
            route(u)
        t_part(units, False)
        return carry

    lax.fori_loop(1, NC, p1, 0)

    wq_cp.wait()
    wv_cp.wait()
    wo_cp.wait()
    r = r_v[:, 0:1, :]
    tok = (lax.broadcasted_iota(jnp.int32, r.shape, 0) * UH
           + lax.broadcasted_iota(jnp.int32, r.shape, 2))
    best = jnp.max(jnp.max(jnp.where(r != r, -jnp.inf, r), axis=0), axis=1, keepdims=True)
    bidx = jnp.min(jnp.min(jnp.where(r == best, tok, S), axis=0), axis=1, keepdims=True)
    idx = jnp.where(bidx == S, 0, bidx)[0, 0]
    rsel = jnp.where(bidx == S, jnp.nan, best)
    base = pl.multiple_of((idx // 16) * 16, 16)
    sel = lax.broadcasted_iota(jnp.int32, (16, 1), 0) == idx - base
    xsel = jnp.sum(jnp.where(sel, x_v[pl.ds(base, 16), :].astype(F32), 0.0), axis=0, keepdims=True)
    xsel_v[...] = jnp.broadcast_to(xsel, (8, D))
    y_v[...] = jnp.zeros_like(y_v)

    put_w_terms(range(7), lambda a: wq_v.at[pl.ds(a // 2 * HD, HD), pl.ds(a % 2 * HD, HD)])
    z_v[...] = jnp.broadcast_to(jnp.sum(z_v[...], axis=1, keepdims=True), z_v.shape)
    same_head = ((lax.broadcasted_iota(jnp.int32, (128, 128), 0) // 16) % 4
                 == lax.broadcasted_iota(jnp.int32, (128, 128), 1) // DH)
    kvs = {}
    for o in range(0, D, 128):
        t = jnp.concatenate([
            jnp.concatenate([t_v[n, pl.ds(o + h, 32, stride=4), :] for h in range(4)], axis=0)
            for n in range(D // 128)], axis=1)
        kvs[o] = jnp.where(same_head, _dot(t.astype(BF16), wv_v[:, o:o + 128]), 0.0).astype(BF16)
    for j in range(0, HD, 128):
        for n in range(0, HD, 256):
            m = [_dot(kvs[o], wo_v[o:o + 128, h + n:h + n + 256]) for o in (j, HD + j) for h in (0, HD)]
            for i, t in enumerate(_rhs_terms(*m)):
                ms_v[i, j // 2:j // 2 + 64, n:n + 256] = _words(t[:64], t[64:])

    def ffn_steps(c):
        st = {}

        def proj(key, w_v, n, k):
            def step():
                p = _dot(xsel_v[:, k:k + HD], w_v[c, k:k + HD, n:n + 128])
                st[key, n] = p if k == 0 else st[key, n] + p
            return step

        def down(n, k):
            def step():
                if k == 0:
                    g = st['g', n]
                    st['h', n] = (g * _sigmoid(g) * st['u', n]).astype(BF16).astype(F32)
                y_v[:, k:k + HD] += _dot(st['h', n], wd_v[c, n:n + 128, k:k + HD])
            return step

        tiles = range(0, FC, 128)
        return ([proj(key, w_v, n, k) for n in tiles for key, w_v in (('g', wg_v), ('u', wu_v)) for k in (0, HD)]
                + [down(n, k) for n in tiles for k in (0, HD)])

    def mix(rows, cols, a, y=None):
        g = jnp.tile(g_v[rows, :], (1, a.shape[1] // 128))
        b = x_v[rows, cols].astype(F32)
        upd = b * 0.0 if y is None else b * 0.0 + y
        out_v[rows, cols] = (g * a + (1.0 - g) * (b + upd)).astype(BF16)

    def p2(c, carry):
        for cp in f_cps(c):
            cp.wait()
        steps = ffn_steps(c) if CFG['FFN'] else []

        def with_ffn(p):
            if steps:
                steps.pop(0)()
            return p

        units = [(idx // U + 1 + c * UC + t) % NU for t in range(UC)]
        for t, u in enumerate(units):
            for m in range(0, HD, MQ):
                rows = slice(m, m + MQ)
                q = _combine({i: with_ffn(proj_term(u, i, rows)) for i in (2, 3, 0, 4, 6, 1, 5)})
                pqn = []
                for qij, o in zip(q, (m, HD + m, m, HD + m)):
                    pq = _phi(qij).reshape(MQ // DH, DH, UH)
                    den = jnp.sum(pq * z_v[o:o + MQ, :].reshape(MQ // DH, DH, UH), axis=1, keepdims=True) + 1e-6
                    pqn.append((pq * (1.0 / den)).reshape(MQ, UH))
                for i, p in enumerate(_lhs_terms(*pqn)):
                    rs_v[t, i, :, rows] = p.T.astype(BF16)
        for t, u in enumerate(units):
            for n in range(0, HD, NA):
                a = _combine({i: with_ffn(_dot(rs_v[t, i], _as_matrix(ms_v[i, :, n:n + NA])))
                              for i in (0, 3, 4, 6, 2, 1, 5)})
                for aij, (i, j) in zip(a, ((0, 0), (0, 1), (1, 0), (1, 1))):
                    cols = slice(j * HD + n, j * HD + n + NA)
                    if t == UC - 1:
                        a_v[i * UH:(i + 1) * UH, cols] = aij
                    mix(pl.ds(pl.multiple_of(u * U + i * UH, UH), UH), cols, aij)
            if t < UC - 1:
                o_cp(u).start()
            else:
                pl.when(c < NC - 1)(o_cp(u).start)
        assert not steps
        return carry

    lax.fori_loop(0, NC, p2, 0)

    y = y_v[:1, :] * _sigmoid(rsel)
    mix(pl.ds(base, 16), slice(None), a_v[pl.ds(pl.multiple_of(base % U, 16), 16), :], jnp.where(sel, y, 0.0))
    o_cp(idx // U).start()
    for u in range(NU):
        o_cp(u).wait()


@jax.jit
def pallas_gated_mix__linear_attn_block__moe_arch_mod__prompt_kernel(
    A_x, A_wqkv, A_wo, B_x, B_w_r, B_w_gate, B_w_up, B_w_down, gate_w,
):
    del B_x
    hbm = pl.BlockSpec(memory_space=pl.ANY)
    vmem = pl.BlockSpec(memory_space=pltpu.VMEM)
    out = pl.pallas_call(
        _body,
        out_shape=jax.ShapeDtypeStruct((S, D), BF16),
        in_specs=[hbm, hbm, hbm, vmem, hbm, hbm, hbm, vmem],
        out_specs=hbm,
        scratch_shapes=[
            pltpu.VMEM((S, D), BF16),
            pltpu.VMEM((2, 2, HD, HD), BF16),
            pltpu.VMEM((D, D), BF16),
            pltpu.VMEM((D, D), BF16),
            pltpu.VMEM((D, D), BF16),
            pltpu.VMEM((NC, D, FC), BF16),
            pltpu.VMEM((NC, D, FC), BF16),
            pltpu.VMEM((NC, FC, D), BF16),
            pltpu.VMEM((7, NU, UH // 2, HD), U32),
            pltpu.VMEM((7, HD // 2, HD), U32),
            pltpu.VMEM((7, HD // 2, UC * UH), U32),
            pltpu.VMEM((D // 128, D, 128), F32),
            pltpu.VMEM((D, 128), F32),
            pltpu.VMEM((7, HD // 2, HD), U32),
            pltpu.VMEM((UC, 7, UH, HD), BF16),
            pltpu.VMEM((16, D), BF16),
            pltpu.VMEM((S // UH, 8, UH), F32),
            pltpu.VMEM((S, 128), F32),
            pltpu.VMEM((U, D), F32),
            pltpu.VMEM((8, D), F32),
            pltpu.VMEM((8, D), F32),
            pltpu.VMEM((S, D), BF16),
            pltpu.SemaphoreType.DMA((NC,)),
            pltpu.SemaphoreType.DMA((7,)),
            pltpu.SemaphoreType.DMA((3, NC)),
            pltpu.SemaphoreType.DMA((NU,)),
        ],
        compiler_params=pltpu.CompilerParams(vmem_limit_bytes=100 * 1024 * 1024),
    )(A_x.reshape(S, D), A_wqkv, A_wo, B_w_r, B_w_gate, B_w_up, B_w_down, gate_w)
    return out.reshape(1, S, D)
```

```python
import jax
import jax.numpy as jnp
from jax import lax
import jax.experimental.pallas as pl
import jax.experimental.pallas.tpu as pltpu

CFG = dict(FFN=1, MQ=512, MT=256, NA=128, EU=2)

S, D, F, DH = 2048, 1024, 3584, 32
HD = D // 2
U = 256
UH = U // 2
NU = S // U
UC = 2
NC = NU // UC
FC = F // NC
F32, BF16, U32 = jnp.float32, jnp.bfloat16, jnp.uint32
NN = (((1,), (0,)), ((), ()))
NT = (((1,), (1,)), ((), ()))


def _dot(a, b, dims=NN):
    return lax.dot_general(a, b, dims, preferred_element_type=F32)


def _phi(t):
    return jnp.where(t > 0, t + 1.0, jnp.exp(t)) + 1e-6


def _sigmoid(t):
    return 1.0 / (1.0 + jnp.exp(-t))


def _lhs_terms(a11, a12, a21, a22):
    return [a11 + a22, a21 + a22, a11, a22, a11 + a12, a21 - a11, a12 - a22]


def _rhs_terms(b11, b12, b21, b22):
    return [b11 + b22, b11, b12 - b22, b21 - b11, b22, b11 + b12, b21 + b22]


def _combine(p):
    return p[0] + p[3] - p[4] + p[6], p[2] + p[4], p[1] + p[3], p[0] - p[1] + p[2] + p[5]


_RHS_AS_LHS = (0, 2, 6, 5, 3, 4, 1)


def _as_matrix(words):
    return pltpu.bitcast(words, BF16)


def _even_odd(mat):
    words = pltpu.bitcast(mat, U32)
    return [pltpu.unpack_elementwise(words, index=i, packed_dtype=BF16, unpacked_dtype=F32) for i in (0, 1)]


def _words(even, odd):
    return pltpu.bitcast(pltpu.pack_elementwise([even, odd], packed_dtype=BF16), U32)


def _words_riffled(v):
    return jnp.concatenate([_words(v[r:r + 64], v[r + 64:r + 128]) for r in range(0, v.shape[0], 128)], axis=0)


def _half(rows):
    return slice(rows.start // 2, rows.stop // 2)


def _body(x_hbm, wqkv_hbm, wo_hbm, wr_ref, wg_hbm, wu_hbm, wd_hbm, gw_ref, out_hbm,
          x_v, wk_v, wq_v, wv_v, wo_v, wg_v, wu_v, wd_v,
          xs_v, ws_v, ps_v, t_v, z_v, ms_v, rs_v, rg_v, r_v, g_v, a_v, xsel_v, y_v, out_v,
          sem_x, sem_w, sem_f, sem_o):
    MQ, MT, NA = CFG['MQ'], CFG['MT'], CFG['NA']

    def x_cp(c):
        rows = pl.ds(c * UC * U, UC * U)
        return pltpu.make_async_copy(x_hbm.at[rows], x_v.at[rows], sem_x.at[c])

    def wk_cp(i, j):
        return pltpu.make_async_copy(wqkv_hbm.at[pl.ds(i * HD, HD), pl.ds(D + j * HD, HD)],
                                     wk_v.at[i, j], sem_w.at[2 * i + j])

    wq_cp = pltpu.make_async_copy(wqkv_hbm.at[:, pl.ds(0, D)], wq_v, sem_w.at[4])
    wv_cp = pltpu.make_async_copy(wqkv_hbm.at[:, pl.ds(2 * D, D)], wv_v, sem_w.at[5])
    wo_cp = pltpu.make_async_copy(wo_hbm, wo_v, sem_w.at[6])

    def f_cps(i):
        hid = pl.ds(pl.multiple_of(i * FC, 128), FC)
        return (pltpu.make_async_copy(wg_hbm.at[:, hid], wg_v.at[i], sem_f.at[0, i]),
                pltpu.make_async_copy(wu_hbm.at[:, hid], wu_v.at[i], sem_f.at[1, i]),
                pltpu.make_async_copy(wd_hbm.at[hid], wd_v.at[i], sem_f.at[2, i]))

    def o_cp(u):
        rows = pl.ds(pl.multiple_of(u * U, U), U)
        return pltpu.make_async_copy(out_v.at[rows], out_hbm.at[rows], sem_o.at[u])

    def make_x_terms(u):
        for n in range(0, HD, 128):
            quads = [x_v[pl.ds(pl.multiple_of(u * U + i * UH, UH), UH), j * HD + n:j * HD + n + 128]
                     for i in (0, 1) for j in (0, 1)]
            even, odd = zip(*[_even_odd(q) for q in quads])
            for i, (e, o) in enumerate(zip(_lhs_terms(*even), _lhs_terms(*odd))):
                xs_v[i, u, :, n:n + 128] = pltpu.bitcast(quads[3 * (i - 2)], U32) if i in (2, 3) else _words(e, o)

    def put_w_terms(which, quadrant):
        pairs = {0: (0, 3, 1), 2: (1, 3, -1), 3: (2, 0, -1), 5: (0, 1, 1), 6: (2, 3, 1)}
        for r in range(0, HD, 128):
            for n in range(0, HD, 128):
                wt = [quadrant(a)[n:n + 128, r:r + 128].T for a in range(4)]
                f = [_even_odd(w) for w in wt]
                for i in which:
                    if i in pairs:
                        a, b, sign = pairs[i]
                        t = _words(*[fa + fb if sign > 0 else fa - fb for fa, fb in zip(f[a], f[b])])
                    else:
                        t = pltpu.bitcast(wt[0 if i == 1 else 3], U32)
                    ws_v[i, r // 2:r // 2 + 64, n:n + 128] = t

    def proj_term(u, i, rows, direct=False):
        if direct and i in (2, 3):
            k = i - 2
            xt = x_v[pl.ds(pl.multiple_of(u * U + k * UH, UH), UH), k * HD:(k + 1) * HD]
        else:
            xt = _as_matrix(xs_v[i, u])
        return _dot(_as_matrix(ws_v[i, _half(rows), :]), xt, NT)

    def route(u, h):
        o = pl.multiple_of(u * U + h * UH, UH)
        rg = _dot(rg_v[...], x_v[pl.ds(o, UH), :], NT)
        r_v[2 * u + h] = rg[:8].astype(BF16).astype(F32)
        g_v[pl.ds(o, UH), :] = jnp.broadcast_to(_sigmoid(rg[1:2]), (UH, UH)).T

    def k_finish(t, rows, prods, first):
        k11, k12, k21, k22 = [_phi(k) for k in _combine(prods)]
        lo, hi = rows, slice(HD + rows.start, HD + rows.stop)
        if first:
            z_v[lo, :] = k11 + k21
            z_v[hi, :] = k12 + k22
        else:
            z_v[lo, :] += k11 + k21
            z_v[hi, :] += k12 + k22
        for i, p in enumerate(_lhs_terms(k11, k21, k12, k22)):
            ps_v[i, _half(rows), t * UH:(t + 1) * UH] = _words_riffled(p)

    def t_part(units, first):
        for m in range(0, HD, MT):
            for n in range(0, HD, 256):
                prods = {}
                for i in (0, 3, 4, 6, 2, 1, 5):
                    rhs = jnp.concatenate([xs_v[_RHS_AS_LHS[i], u, :, n:n + 256] for u in units], axis=0)
                    prods[i] = _dot(_as_matrix(ps_v[i, m // 2:(m + MT) // 2, :]), _as_matrix(rhs))
                for t, (i, j) in zip(_combine(prods), ((0, 0), (0, 1), (1, 0), (1, 1))):
                    rows = slice(i * HD + m, i * HD + m + MT)
                    for k in (0, 128):
                        if first:
                            t_v[(j * HD + n + k) // 128, rows, :] = t[:, k:k + 128]
                        else:
                            t_v[(j * HD + n + k) // 128, rows, :] += t[:, k:k + 128]

    x_cp(0).start()
    wk_cp(0, 0).start()
    wk_cp(1, 1).start()
    r16 = lax.broadcasted_iota(jnp.int32, (16, D), 0)
    wr = wr_ref[...].astype(F32).reshape(1, D)
    gw = gw_ref[...].astype(F32).reshape(1, D)
    rg_v[...] = jnp.where(r16 == 0, wr, jnp.where(r16 == 1, gw, 0.0)).astype(BF16)
    x_cp(0).wait()
    wk_cp(0, 0).wait()
    wk_cp(1, 1).wait()
    wk_cp(0, 1).start()
    wk_cp(1, 0).start()
    put_w_terms((1, 4, 0), lambda a: wk_v.at[a // 2, a // 2])
    full = slice(0, HD)
    for u in range(UC):
        make_x_terms(u)
    early = [{i: proj_term(u, i, full) for i in (1, 4, 0)} for u in range(CFG['EU'])]
    wk_cp(0, 1).wait()
    wk_cp(1, 0).wait()
    for c in range(1, NC):
        x_cp(c).start()
    put_w_terms((3, 6, 2, 5), lambda a: wk_v.at[a // 2, a % 2])
    early += [{i: proj_term(u, i, full) for i in (1, 4, 0)} for u in range(CFG['EU'], UC)]
    for u in range(UC):
        for n, i in enumerate((3, 6, 2, 5)):
            early[u][i] = proj_term(u, i, full)
            if n < 2:
                route(u, n)
        k_finish(u, full, early[u], u == 0)
    t_part(range(UC), True)
    for c in range(1, NC):
        x_cp(c).wait()
    for cp in (wq_cp, wv_cp, wo_cp) + f_cps(0):
        cp.start()

    def p1(c, carry):
        for cp in f_cps(c):
            cp.start()
        units = [c * UC + t for t in range(UC)]
        for u in units:
            make_x_terms(u)
        for t, u in enumerate(units):
            prods = {}
            for n, i in enumerate((2, 3, 0, 4, 6, 1, 5)):
                prods[i] = proj_term(u, i, full, True)
                if n in (2, 4):
                    route(u, n // 2 - 1)
            k_finish(t, full, prods, False)
        t_part(units, False)
        return carry

    lax.fori_loop(1, NC, p1, 0)

    wq_cp.wait()
    wv_cp.wait()
    wo_cp.wait()
    r = r_v[:, 0:1, :]
    tok = (lax.broadcasted_iota(jnp.int32, r.shape, 0) * UH
           + lax.broadcasted_iota(jnp.int32, r.shape, 2))
    best = jnp.max(jnp.max(jnp.where(r != r, -jnp.inf, r), axis=0), axis=1, keepdims=True)
    bidx = jnp.min(jnp.min(jnp.where(r == best, tok, S), axis=0), axis=1, keepdims=True)
    idx = jnp.where(bidx == S, 0, bidx)[0, 0]
    rsel = jnp.where(bidx == S, jnp.nan, best)
    base = pl.multiple_of((idx // 16) * 16, 16)
    sel = lax.broadcasted_iota(jnp.int32, (16, 1), 0) == idx - base
    xsel = jnp.sum(jnp.where(sel, x_v[pl.ds(base, 16), :].astype(F32), 0.0), axis=0, keepdims=True)
    xsel_v[...] = jnp.broadcast_to(xsel, (8, D))
    y_v[...] = jnp.zeros_like(y_v)

    put_w_terms(range(7), lambda a: wq_v.at[pl.ds(a // 2 * HD, HD), pl.ds(a % 2 * HD, HD)])
    z_v[...] = jnp.broadcast_to(jnp.sum(z_v[...], axis=1, keepdims=True), z_v.shape)
    same_head = ((lax.broadcasted_iota(jnp.int32, (128, 128), 0) // 16) % 4
                 == lax.broadcasted_iota(jnp.int32, (128, 128), 1) // DH)
    kvs = {}
    for o in range(0, D, 128):
        t = jnp.concatenate([
            jnp.concatenate([t_v[n, pl.ds(o + h, 32, stride=4), :] for h in range(4)], axis=0)
            for n in range(D // 128)], axis=1)
        kvs[o] = jnp.where(same_head, _dot(t.astype(BF16), wv_v[:, o:o + 128]), 0.0).astype(BF16)
    for j in range(0, HD, 128):
        for n in range(0, HD, 256):
            m = [_dot(kvs[o], wo_v[o:o + 128, h + n:h + n + 256]) for o in (j, HD + j) for h in (0, HD)]
            for i, t in enumerate(_rhs_terms(*m)):
                ms_v[i, j // 2:j // 2 + 64, n:n + 256] = _words(t[:64], t[64:])

    def ffn_steps(c):
        st = {}

        def proj(key, w_v, n, k):
            def step():
                p = _dot(xsel_v[:, k:k + HD], w_v[c, k:k + HD, n:n + 128])
                st[key, n] = p if k == 0 else st[key, n] + p
            return step

        def down(n, k):
            def step():
                if k == 0:
                    g = st['g', n]
                    st['h', n] = (g * _sigmoid(g) * st['u', n]).astype(BF16).astype(F32)
                y_v[:, k:k + HD] += _dot(st['h', n], wd_v[c, n:n + 128, k:k + HD])
            return step

        tiles = range(0, FC, 128)
        return ([proj(key, w_v, n, k) for n in tiles for key, w_v in (('g', wg_v), ('u', wu_v)) for k in (0, HD)]
                + [down(n, k) for n in tiles for k in (0, HD)])

    def mix(rows, cols, a, y=None):
        g = jnp.tile(g_v[rows, :], (1, a.shape[1] // 128))
        b = x_v[rows, cols].astype(F32)
        upd = b * 0.0 if y is None else b * 0.0 + y
        out_v[rows, cols] = (g * a + (1.0 - g) * (b + upd)).astype(BF16)

    def p2(c, carry):
        for cp in f_cps(c):
            cp.wait()
        steps = ffn_steps(c) if CFG['FFN'] else []

        def with_ffn(p):
            if steps:
                steps.pop(0)()
            return p

        units = [(idx // U + 1 + c * UC + t) % NU for t in range(UC)]
        for t, u in enumerate(units):
            for m in range(0, HD, MQ):
                rows = slice(m, m + MQ)
                q = _combine({i: with_ffn(proj_term(u, i, rows)) for i in (2, 3, 0, 4, 6, 1, 5)})
                pqn = []
                for qij, o in zip(q, (m, HD + m, m, HD + m)):
                    pq = _phi(qij).reshape(MQ // DH, DH, UH)
                    den = jnp.sum(pq * z_v[o:o + MQ, :].reshape(MQ // DH, DH, UH), axis=1, keepdims=True) + 1e-6
                    pqn.append((pq * (1.0 / den)).reshape(MQ, UH))
                for i, p in enumerate(_lhs_terms(*pqn)):
                    rs_v[t, i, :, rows] = p.T.astype(BF16)
        for t, u in enumerate(units):
            for n in range(0, HD, NA):
                a = _combine({i: with_ffn(_dot(rs_v[t, i], _as_matrix(ms_v[i, :, n:n + NA])))
                              for i in (0, 3, 4, 6, 2, 1, 5)})
                for aij, (i, j) in zip(a, ((0, 0), (0, 1), (1, 0), (1, 1))):
                    cols = slice(j * HD + n, j * HD + n + NA)
                    if t == UC - 1:
                        a_v[i * UH:(i + 1) * UH, cols] = aij
                    mix(pl.ds(pl.multiple_of(u * U + i * UH, UH), UH), cols, aij)
            if t < UC - 1:
                o_cp(u).start()
            else:
                pl.when(c < NC - 1)(o_cp(u).start)
        assert not steps
        return carry

    lax.fori_loop(0, NC, p2, 0)

    y = y_v[:1, :] * _sigmoid(rsel)
    mix(pl.ds(base, 16), slice(None), a_v[pl.ds(pl.multiple_of(base % U, 16), 16), :], jnp.where(sel, y, 0.0))
    o_cp(idx // U).start()
    for u in range(NU):
        o_cp(u).wait()


@jax.jit
def pallas_gated_mix__linear_attn_block__moe_arch_mod__prompt_kernel(
    A_x, A_wqkv, A_wo, B_x, B_w_r, B_w_gate, B_w_up, B_w_down, gate_w,
):
    del B_x
    hbm = pl.BlockSpec(memory_space=pl.ANY)
    vmem = pl.BlockSpec(memory_space=pltpu.VMEM)
    out = pl.pallas_call(
        _body,
        out_shape=jax.ShapeDtypeStruct((S, D), BF16),
        in_specs=[hbm, hbm, hbm, vmem, hbm, hbm, hbm, vmem],
        out_specs=hbm,
        scratch_shapes=[
            pltpu.VMEM((S, D), BF16),
            pltpu.VMEM((2, 2, HD, HD), BF16),
            pltpu.VMEM((D, D), BF16),
            pltpu.VMEM((D, D), BF16),
            pltpu.VMEM((D, D), BF16),
            pltpu.VMEM((NC, D, FC), BF16),
            pltpu.VMEM((NC, D, FC), BF16),
            pltpu.VMEM((NC, FC, D), BF16),
            pltpu.VMEM((7, NU, UH // 2, HD), U32),
            pltpu.VMEM((7, HD // 2, HD), U32),
            pltpu.VMEM((7, HD // 2, UC * UH), U32),
            pltpu.VMEM((D // 128, D, 128), F32),
            pltpu.VMEM((D, 128), F32),
            pltpu.VMEM((7, HD // 2, HD), U32),
            pltpu.VMEM((UC, 7, UH, HD), BF16),
            pltpu.VMEM((16, D), BF16),
            pltpu.VMEM((S // UH, 8, UH), F32),
            pltpu.VMEM((S, 128), F32),
            pltpu.VMEM((U, D), F32),
            pltpu.VMEM((8, D), F32),
            pltpu.VMEM((8, D), F32),
            pltpu.VMEM((S, D), BF16),
            pltpu.SemaphoreType.DMA((NC,)),
            pltpu.SemaphoreType.DMA((7,)),
            pltpu.SemaphoreType.DMA((3, NC)),
            pltpu.SemaphoreType.DMA((NU,)),
        ],
        compiler_params=pltpu.CompilerParams(vmem_limit_bytes=100 * 1024 * 1024),
    )(A_x.reshape(S, D), A_wqkv, A_wo, B_w_r, B_w_gate, B_w_up, B_w_down, gate_w)
    return out.reshape(1, S, D)
```

```python
import jax
import jax.numpy as jnp
from jax import lax
import jax.experimental.pallas as pl
import jax.experimental.pallas.tpu as pltpu

CFG = dict(FFN=1, MQ=512, MT=256, NA=128, OW=256)

S, D, F, DH = 2048, 1024, 3584, 32
HD = D // 2
U = 256
UH = U // 2
NU = S // U
UC = 2
NC = NU // UC
FC = F // NC
F32, BF16, U32 = jnp.float32, jnp.bfloat16, jnp.uint32
NN = (((1,), (0,)), ((), ()))
NT = (((1,), (1,)), ((), ()))


def _dot(a, b, dims=NN):
    return lax.dot_general(a, b, dims, preferred_element_type=F32)


def _phi(t):
    return jnp.where(t > 0, t + 1.0, jnp.exp(t)) + 1e-6


def _sigmoid(t):
    return 1.0 / (1.0 + jnp.exp(-t))


def _lhs_terms(a11, a12, a21, a22):
    return [a11 + a22, a21 + a22, a11, a22, a11 + a12, a21 - a11, a12 - a22]


def _rhs_terms(b11, b12, b21, b22):
    return [b11 + b22, b11, b12 - b22, b21 - b11, b22, b11 + b12, b21 + b22]


def _combine(p):
    return p[0] + p[3] - p[4] + p[6], p[2] + p[4], p[1] + p[3], p[0] - p[1] + p[2] + p[5]


_RHS_AS_LHS = (0, 2, 6, 5, 3, 4, 1)


def _as_matrix(words):
    return pltpu.bitcast(words, BF16)


def _even_odd(mat):
    words = pltpu.bitcast(mat, U32)
    return [pltpu.unpack_elementwise(words, index=i, packed_dtype=BF16, unpacked_dtype=F32) for i in (0, 1)]


def _words(even, odd):
    return pltpu.bitcast(pltpu.pack_elementwise([even, odd], packed_dtype=BF16), U32)


def _words_riffled(v):
    return jnp.concatenate([_words(v[r:r + 64], v[r + 64:r + 128]) for r in range(0, v.shape[0], 128)], axis=0)


def _half(rows):
    return slice(rows.start // 2, rows.stop // 2)


def _body(x_hbm, wqkv_hbm, wo_hbm, wr_ref, wg_hbm, wu_hbm, wd_hbm, gw_ref, out_hbm,
          x_v, wk_v, wq_v, wv_v, wo_v, wg_v, wu_v, wd_v,
          xs_v, ws_v, ps_v, t_v, z_v, ms_v, rs_v, rg_v, r_v, g_v, xsel_v, y_v, out_v,
          sem_x, sem_w, sem_f, sem_o, sem_s):
    MQ, MT, NA, OW = CFG['MQ'], CFG['MT'], CFG['NA'], CFG['OW']

    def x_cp(c):
        rows = pl.ds(c * UC * U, UC * U)
        return pltpu.make_async_copy(x_hbm.at[rows], x_v.at[rows], sem_x.at[c])

    def wk_cp(i, j):
        return pltpu.make_async_copy(wqkv_hbm.at[pl.ds(i * HD, HD), pl.ds(D + j * HD, HD)],
                                     wk_v.at[i, j], sem_w.at[2 * i + j])

    wq_cp = pltpu.make_async_copy(wqkv_hbm.at[:, pl.ds(0, D)], wq_v, sem_w.at[4])
    wv_cp = pltpu.make_async_copy(wqkv_hbm.at[:, pl.ds(2 * D, D)], wv_v, sem_w.at[5])
    wo_cp = pltpu.make_async_copy(wo_hbm, wo_v, sem_w.at[6])

    def f_cps(i):
        hid = pl.ds(pl.multiple_of(i * FC, 128), FC)
        return (pltpu.make_async_copy(wg_hbm.at[:, hid], wg_v.at[i], sem_f.at[0, i]),
                pltpu.make_async_copy(wu_hbm.at[:, hid], wu_v.at[i], sem_f.at[1, i]),
                pltpu.make_async_copy(wd_hbm.at[hid], wd_v.at[i], sem_f.at[2, i]))

    def out_cps(c, t, u, n=0):
        rows = pl.ds(pl.multiple_of(u * U, U), U)
        if t < UC - 1:
            return [pltpu.make_async_copy(out_v.at[rows], out_hbm.at[rows], sem_o.at[c, 0])]
        return [pltpu.make_async_copy(out_v.at[rows, pl.ds(j * HD + n, OW)], out_hbm.at[rows, pl.ds(j * HD + n, OW)],
                                      sem_o.at[c, 1 + 2 * (n // OW) + j]) for j in (0, 1)]

    def make_x_terms(u):
        for n in range(0, HD, 128):
            quads = [x_v[pl.ds(pl.multiple_of(u * U + i * UH, UH), UH), j * HD + n:j * HD + n + 128]
                     for i in (0, 1) for j in (0, 1)]
            even, odd = zip(*[_even_odd(q) for q in quads])
            for i, (e, o) in enumerate(zip(_lhs_terms(*even), _lhs_terms(*odd))):
                xs_v[i, u, :, n:n + 128] = pltpu.bitcast(quads[3 * (i - 2)], U32) if i in (2, 3) else _words(e, o)

    def put_w_terms(which, quadrant):
        pairs = {0: (0, 3, 1), 2: (1, 3, -1), 3: (2, 0, -1), 5: (0, 1, 1), 6: (2, 3, 1)}
        for r in range(0, HD, 128):
            for n in range(0, HD, 128):
                wt = [quadrant(a)[n:n + 128, r:r + 128].T for a in range(4)]
                f = [_even_odd(w) for w in wt]
                for i in which:
                    if i in pairs:
                        a, b, sign = pairs[i]
                        t = _words(*[fa + fb if sign > 0 else fa - fb for fa, fb in zip(f[a], f[b])])
                    else:
                        t = pltpu.bitcast(wt[0 if i == 1 else 3], U32)
                    ws_v[i, r // 2:r // 2 + 64, n:n + 128] = t

    def proj_term(u, i, rows, direct=False):
        if direct and i in (2, 3):
            k = i - 2
            xt = x_v[pl.ds(pl.multiple_of(u * U + k * UH, UH), UH), k * HD:(k + 1) * HD]
        else:
            xt = _as_matrix(xs_v[i, u])
        return _dot(_as_matrix(ws_v[i, _half(rows), :]), xt, NT)

    def route(u, h):
        o = pl.multiple_of(u * U + h * UH, UH)
        rg = _dot(rg_v[...], x_v[pl.ds(o, UH), :], NT)
        r_v[2 * u + h] = rg[:8].astype(BF16).astype(F32)
        g_v[pl.ds(o, UH), :] = jnp.broadcast_to(_sigmoid(rg[1:2]), (UH, UH)).T

    def k_finish(t, rows, prods, first):
        k11, k12, k21, k22 = [_phi(k) for k in _combine(prods)]
        lo, hi = rows, slice(HD + rows.start, HD + rows.stop)
        if first:
            z_v[lo, :] = k11 + k21
            z_v[hi, :] = k12 + k22
        else:
            z_v[lo, :] += k11 + k21
            z_v[hi, :] += k12 + k22
        for i, p in enumerate(_lhs_terms(k11, k21, k12, k22)):
            ps_v[i, _half(rows), t * UH:(t + 1) * UH] = _words_riffled(p)

    def t_part(units, first):
        for m in range(0, HD, MT):
            for n in range(0, HD, 256):
                prods = {}
                for i in (0, 3, 4, 6, 2, 1, 5):
                    rhs = jnp.concatenate([xs_v[_RHS_AS_LHS[i], u, :, n:n + 256] for u in units], axis=0)
                    prods[i] = _dot(_as_matrix(ps_v[i, m // 2:(m + MT) // 2, :]), _as_matrix(rhs))
                for t, (i, j) in zip(_combine(prods), ((0, 0), (0, 1), (1, 0), (1, 1))):
                    rows = slice(i * HD + m, i * HD + m + MT)
                    for k in (0, 128):
                        if first:
                            t_v[(j * HD + n + k) // 128, rows, :] = t[:, k:k + 128]
                        else:
                            t_v[(j * HD + n + k) // 128, rows, :] += t[:, k:k + 128]

    x0 = [pltpu.make_async_copy(x_hbm.at[pl.ds(u * U, U)], x_v.at[pl.ds(u * U, U)], sem_s.at[u]) for u in (0, 1)]
    w22 = [pltpu.make_async_copy(wqkv_hbm.at[pl.ds(HD + h, HD // 2), pl.ds(D + HD, HD)],
                                 wk_v.at[1, 1, pl.ds(h, HD // 2)], sem_s.at[2 + h // (HD // 2)])
           for h in (0, HD // 2)]
    for cp in (x0[0], wk_cp(0, 0), *w22):
        cp.start()
    r16 = lax.broadcasted_iota(jnp.int32, (16, D), 0)
    wr = wr_ref[...].astype(F32).reshape(1, D)
    gw = gw_ref[...].astype(F32).reshape(1, D)
    rg_v[...] = jnp.where(r16 == 0, wr, jnp.where(r16 == 1, gw, 0.0)).astype(BF16)
    w22[0].wait()
    for cp in (x0[1], wk_cp(0, 1), wk_cp(1, 0)):
        cp.start()
    for cp in (w22[1], x0[0], wk_cp(0, 0)):
        cp.wait()
    put_w_terms((1, 4, 0), lambda a: wk_v.at[a // 2, a // 2])
    full = slice(0, HD)
    make_x_terms(0)
    early = [{i: proj_term(0, i, full) for i in (1, 4, 0)}]
    for h in (0, 1):
        route(0, h)
    for cp in (x0[1], wk_cp(0, 1), wk_cp(1, 0)):
        cp.wait()
    for c in range(1, NC):
        x_cp(c).start()
    make_x_terms(1)
    put_w_terms((3, 6, 2, 5), lambda a: wk_v.at[a // 2, a % 2])
    early.append({i: proj_term(1, i, full) for i in (1, 4, 0)})
    for u in range(UC):
        for n, i in enumerate((3, 6, 2, 5)):
            early[u][i] = proj_term(u, i, full)
            if u == 1 and n < 2:
                route(u, n)
        k_finish(u, full, early[u], u == 0)
    t_part(range(UC), True)
    for c in range(1, NC):
        x_cp(c).wait()
    for cp in (wq_cp, wv_cp, wo_cp) + f_cps(0):
        cp.start()

    def p1(c, carry):
        for cp in f_cps(c):
            cp.start()
        units = [c * UC + t for t in range(UC)]
        for u in units:
            make_x_terms(u)
        for t, u in enumerate(units):
            prods = {}
            for n, i in enumerate((2, 3, 0, 4, 6, 1, 5)):
                prods[i] = proj_term(u, i, full, True)
                if n in (2, 4):
                    route(u, n // 2 - 1)
            k_finish(t, full, prods, False)
        t_part(units, False)
        return carry

    lax.fori_loop(1, NC, p1, 0)

    wq_cp.wait()
    wv_cp.wait()
    wo_cp.wait()
    r = r_v[:, 0:1, :]
    tok = (lax.broadcasted_iota(jnp.int32, r.shape, 0) * UH
           + lax.broadcasted_iota(jnp.int32, r.shape, 2))
    best = jnp.max(jnp.max(jnp.where(r != r, -jnp.inf, r), axis=0), axis=1, keepdims=True)
    bidx = jnp.min(jnp.min(jnp.where(r == best, tok, S), axis=0), axis=1, keepdims=True)
    idx = jnp.where(bidx == S, 0, bidx)[0, 0]
    rsel = jnp.where(bidx == S, jnp.nan, best)
    base = pl.multiple_of((idx // 16) * 16, 16)
    sel = lax.broadcasted_iota(jnp.int32, (16, 1), 0) == idx - base
    xsel = jnp.sum(jnp.where(sel, x_v[pl.ds(base, 16), :].astype(F32), 0.0), axis=0, keepdims=True)
    xsel_v[...] = jnp.broadcast_to(xsel, (8, D))
    y_v[...] = jnp.zeros_like(y_v)

    put_w_terms(range(7), lambda a: wq_v.at[pl.ds(a // 2 * HD, HD), pl.ds(a % 2 * HD, HD)])
    z_v[...] = jnp.broadcast_to(jnp.sum(z_v[...], axis=1, keepdims=True), z_v.shape)
    same_head = ((lax.broadcasted_iota(jnp.int32, (128, 128), 0) // 16) % 4
                 == lax.broadcasted_iota(jnp.int32, (128, 128), 1) // DH)
    kvs = {}
    for o in range(0, D, 128):
        t = jnp.concatenate([
            jnp.concatenate([t_v[n, pl.ds(o + h, 32, stride=4), :] for h in range(4)], axis=0)
            for n in range(D // 128)], axis=1)
        kvs[o] = jnp.where(same_head, _dot(t.astype(BF16), wv_v[:, o:o + 128]), 0.0).astype(BF16)
    for j in range(0, HD, 128):
        for n in range(0, HD, 256):
            m = [_dot(kvs[o], wo_v[o:o + 128, h + n:h + n + 256]) for o in (j, HD + j) for h in (0, HD)]
            for i, t in enumerate(_rhs_terms(*m)):
                ms_v[i, j // 2:j // 2 + 64, n:n + 256] = _words(t[:64], t[64:])

    def ffn_steps(c):
        st = {}

        def proj(key, w_v, n, k):
            def step():
                p = _dot(xsel_v[:, k:k + HD], w_v[c, k:k + HD, n:n + 128])
                st[key, n] = p if k == 0 else st[key, n] + p
            return step

        def down(n, k):
            def step():
                if k == 0:
                    g = st['g', n]
                    st['h', n] = (g * _sigmoid(g) * st['u', n]).astype(BF16).astype(F32)
                y_v[:, k:k + HD] += _dot(st['h', n], wd_v[c, n:n + 128, k:k + HD])
            return step

        tiles = range(0, FC, 128)
        return ([proj(key, w_v, n, k) for n in tiles for key, w_v in (('g', wg_v), ('u', wu_v)) for k in (0, HD)]
                + [down(n, k) for n in tiles for k in (0, HD)])

    def unit(c, t):
        return (idx // U + 1 + c * UC + t) % NU

    def p2(c, carry):
        for cp in f_cps(c):
            cp.wait()
        steps = ffn_steps(c) if CFG['FFN'] else []

        def with_ffn(p):
            if steps:
                steps.pop(0)()
            return p

        units = [unit(c, t) for t in range(UC)]
        for t, u in enumerate(units):
            for m in range(0, HD, MQ):
                rows = slice(m, m + MQ)
                q = _combine({i: with_ffn(proj_term(u, i, rows)) for i in (2, 3, 0, 4, 6, 1, 5)})
                pqn = []
                for qij, o in zip(q, (m, HD + m, m, HD + m)):
                    pq = _phi(qij).reshape(MQ // DH, DH, UH)
                    den = jnp.sum(pq * z_v[o:o + MQ, :].reshape(MQ // DH, DH, UH), axis=1, keepdims=True) + 1e-6
                    pqn.append((pq * (1.0 / den)).reshape(MQ, UH))
                for i, p in enumerate(_lhs_terms(*pqn)):
                    rs_v[t, i, :, rows] = p.T.astype(BF16)
        y = None
        for t, u in enumerate(units):
            if t == UC - 1:
                assert not steps
                y = y_v[:1, :] * _sigmoid(rsel)
            for n in range(0, HD, NA):
                a = _combine({i: with_ffn(_dot(rs_v[t, i], _as_matrix(ms_v[i, :, n:n + NA])))
                              for i in (0, 3, 4, 6, 2, 1, 5)})
                for aij, (i, j) in zip(a, ((0, 0), (0, 1), (1, 0), (1, 1))):
                    o = pl.multiple_of(u * U + i * UH, UH)
                    rows, cols = pl.ds(o, UH), slice(j * HD + n, j * HD + n + NA)
                    g = jnp.tile(g_v[rows, :], (1, NA // 128))
                    b = x_v[rows, cols].astype(F32)
                    upd = b * 0.0
                    if y is not None:
                        hit = lax.broadcasted_iota(jnp.int32, (UH, NA), 0) == idx - o
                        upd = upd + jnp.where(hit, y[:, cols], 0.0)
                    out_v[rows, cols] = (g * aij + (1.0 - g) * (b + upd)).astype(BF16)
                if t == UC - 1 and (n + NA) % OW == 0:
                    for cp in out_cps(c, t, u, n + NA - OW):
                        cp.start()
            if t < UC - 1:
                for cp in out_cps(c, t, u):
                    cp.start()
        return carry

    lax.fori_loop(0, NC, p2, 0)
    for c in range(NC):
        for t in range(UC):
            for n in range(0, HD if t == UC - 1 else 1, OW):
                for cp in out_cps(c, t, unit(c, t), n):
                    cp.wait()


@jax.jit
def pallas_gated_mix__linear_attn_block__moe_arch_mod__prompt_kernel(
    A_x, A_wqkv, A_wo, B_x, B_w_r, B_w_gate, B_w_up, B_w_down, gate_w,
):
    del B_x
    hbm = pl.BlockSpec(memory_space=pl.ANY)
    vmem = pl.BlockSpec(memory_space=pltpu.VMEM)
    out = pl.pallas_call(
        _body,
        out_shape=jax.ShapeDtypeStruct((S, D), BF16),
        in_specs=[hbm, hbm, hbm, vmem, hbm, hbm, hbm, vmem],
        out_specs=hbm,
        scratch_shapes=[
            pltpu.VMEM((S, D), BF16),
            pltpu.VMEM((2, 2, HD, HD), BF16),
            pltpu.VMEM((D, D), BF16),
            pltpu.VMEM((D, D), BF16),
            pltpu.VMEM((D, D), BF16),
            pltpu.VMEM((NC, D, FC), BF16),
            pltpu.VMEM((NC, D, FC), BF16),
            pltpu.VMEM((NC, FC, D), BF16),
            pltpu.VMEM((7, NU, UH // 2, HD), U32),
            pltpu.VMEM((7, HD // 2, HD), U32),
            pltpu.VMEM((7, HD // 2, UC * UH), U32),
            pltpu.VMEM((D // 128, D, 128), F32),
            pltpu.VMEM((D, 128), F32),
            pltpu.VMEM((7, HD // 2, HD), U32),
            pltpu.VMEM((UC, 7, UH, HD), BF16),
            pltpu.VMEM((16, D), BF16),
            pltpu.VMEM((S // UH, 8, UH), F32),
            pltpu.VMEM((S, 128), F32),
            pltpu.VMEM((8, D), F32),
            pltpu.VMEM((8, D), F32),
            pltpu.VMEM((S, D), BF16),
            pltpu.SemaphoreType.DMA((NC,)),
            pltpu.SemaphoreType.DMA((7,)),
            pltpu.SemaphoreType.DMA((3, NC)),
            pltpu.SemaphoreType.DMA((NC, 1 + 2 * HD // CFG['OW'])),
            pltpu.SemaphoreType.DMA((4,)),
        ],
        compiler_params=pltpu.CompilerParams(vmem_limit_bytes=100 * 1024 * 1024),
    )(A_x.reshape(S, D), A_wqkv, A_wo, B_w_r, B_w_gate, B_w_up, B_w_down, gate_w)
    return out.reshape(1, S, D)
```

```python
import jax
import jax.numpy as jnp
from jax import lax
import jax.experimental.pallas as pl
import jax.experimental.pallas.tpu as pltpu

S, D, F, DH = 2048, 1024, 3584, 32
HD = D // 2
U = 256
UH = U // 2
NU = S // U
UC = 2
NC = NU // UC
FC = F // NC
MT = 256
OW = 256
F32, BF16, U32 = jnp.float32, jnp.bfloat16, jnp.uint32
NN = (((1,), (0,)), ((), ()))
NT = (((1,), (1,)), ((), ()))


def _dot(a, b, dims=NN):
    return lax.dot_general(a, b, dims, preferred_element_type=F32)


def _phi(t):
    return jnp.where(t > 0, t + 1.0, jnp.exp(t)) + 1e-6


def _sigmoid(t):
    return 1.0 / (1.0 + jnp.exp(-t))


def _lhs_terms(a11, a12, a21, a22):
    return [a11 + a22, a21 + a22, a11, a22, a11 + a12, a21 - a11, a12 - a22]


def _rhs_terms(b11, b12, b21, b22):
    return [b11 + b22, b11, b12 - b22, b21 - b11, b22, b11 + b12, b21 + b22]


def _combine(p):
    return p[0] + p[3] - p[4] + p[6], p[2] + p[4], p[1] + p[3], p[0] - p[1] + p[2] + p[5]


_RHS_AS_LHS = (0, 2, 6, 5, 3, 4, 1)


def _as_matrix(words):
    return pltpu.bitcast(words, BF16)


def _even_odd(mat):
    words = pltpu.bitcast(mat, U32)
    return [pltpu.unpack_elementwise(words, index=i, packed_dtype=BF16, unpacked_dtype=F32) for i in (0, 1)]


def _words(even, odd):
    return pltpu.bitcast(pltpu.pack_elementwise([even, odd], packed_dtype=BF16), U32)


def _words_riffled(v):
    return jnp.concatenate([_words(v[r:r + 64], v[r + 64:r + 128]) for r in range(0, v.shape[0], 128)], axis=0)


def _body(x_hbm, wqkv_hbm, wo_hbm, wr_ref, wg_hbm, wu_hbm, wd_hbm, gw_ref, out_hbm,
          x_v, wk_v, wq_v, wv_v, wo_v, wg_v, wu_v, wd_v,
          xs_v, ws_v, ps_v, t_v, z_v, ms_v, rs_v, rg_v, r_v, g_v, xsel_v, y_v, out_v,
          sem_x, sem_w, sem_f, sem_o, sem_s):
    def x_cp(c):
        rows = pl.ds(c * UC * U, UC * U)
        return pltpu.make_async_copy(x_hbm.at[rows], x_v.at[rows], sem_x.at[c])

    def wk_cp(i, j):
        return pltpu.make_async_copy(wqkv_hbm.at[pl.ds(i * HD, HD), pl.ds(D + j * HD, HD)],
                                     wk_v.at[i, j], sem_w.at[2 * i + j])

    wq_cp = pltpu.make_async_copy(wqkv_hbm.at[:, pl.ds(0, D)], wq_v, sem_w.at[4])
    wv_cp = pltpu.make_async_copy(wqkv_hbm.at[:, pl.ds(2 * D, D)], wv_v, sem_w.at[5])
    wo_cp = pltpu.make_async_copy(wo_hbm, wo_v, sem_w.at[6])

    def f_cps(i):
        hid = pl.ds(pl.multiple_of(i * FC, 128), FC)
        return (pltpu.make_async_copy(wg_hbm.at[:, hid], wg_v.at[i], sem_f.at[0, i]),
                pltpu.make_async_copy(wu_hbm.at[:, hid], wu_v.at[i], sem_f.at[1, i]),
                pltpu.make_async_copy(wd_hbm.at[hid], wd_v.at[i], sem_f.at[2, i]))

    def out_cps(c, t, u, n=0):
        rows = pl.ds(pl.multiple_of(u * U, U), U)
        if t < UC - 1:
            return [pltpu.make_async_copy(out_v.at[rows], out_hbm.at[rows], sem_o.at[c, 0])]
        return [pltpu.make_async_copy(out_v.at[rows, pl.ds(j * HD + n, OW)], out_hbm.at[rows, pl.ds(j * HD + n, OW)],
                                      sem_o.at[c, 1 + 2 * (n // OW) + j]) for j in (0, 1)]

    def make_x_terms(u):
        for n in range(0, HD, 128):
            quads = [x_v[pl.ds(pl.multiple_of(u * U + i * UH, UH), UH), j * HD + n:j * HD + n + 128]
                     for i in (0, 1) for j in (0, 1)]
            even, odd = zip(*[_even_odd(q) for q in quads])
            for i, (e, o) in enumerate(zip(_lhs_terms(*even), _lhs_terms(*odd))):
                xs_v[i, u, :, n:n + 128] = pltpu.bitcast(quads[3 * (i - 2)], U32) if i in (2, 3) else _words(e, o)

    def put_w_terms(which, quadrant):
        pairs = {0: (0, 3, 1), 2: (1, 3, -1), 3: (2, 0, -1), 5: (0, 1, 1), 6: (2, 3, 1)}
        for r in range(0, HD, 128):
            for n in range(0, HD, 128):
                wt = [quadrant(a)[n:n + 128, r:r + 128].T for a in range(4)]
                f = [_even_odd(w) for w in wt]
                for i in which:
                    if i in pairs:
                        a, b, sign = pairs[i]
                        t = _words(*[fa + fb if sign > 0 else fa - fb for fa, fb in zip(f[a], f[b])])
                    else:
                        t = pltpu.bitcast(wt[0 if i == 1 else 3], U32)
                    ws_v[i, r // 2:r // 2 + 64, n:n + 128] = t

    def proj_term(u, i, direct=False):
        if direct and i in (2, 3):
            k = i - 2
            xt = x_v[pl.ds(pl.multiple_of(u * U + k * UH, UH), UH), k * HD:(k + 1) * HD]
        else:
            xt = _as_matrix(xs_v[i, u])
        return _dot(_as_matrix(ws_v[i]), xt, NT)

    def route(u, h):
        o = pl.multiple_of(u * U + h * UH, UH)
        rg = _dot(rg_v[...], x_v[pl.ds(o, UH), :], NT)
        r_v[2 * u + h] = rg[:8].astype(BF16).astype(F32)
        g_v[pl.ds(o, UH), :] = jnp.broadcast_to(_sigmoid(rg[1:2]), (UH, UH)).T

    def k_finish(t, prods, first):
        k11, k12, k21, k22 = [_phi(k) for k in _combine(prods)]
        if first:
            z_v[:HD, :] = k11 + k21
            z_v[HD:, :] = k12 + k22
        else:
            z_v[:HD, :] += k11 + k21
            z_v[HD:, :] += k12 + k22
        for i, p in enumerate(_lhs_terms(k11, k21, k12, k22)):
            ps_v[i, :, t * UH:(t + 1) * UH] = _words_riffled(p)

    def t_part(units, first):
        for m in range(0, HD, MT):
            for n in range(0, HD, 256):
                prods = {}
                for i in (0, 3, 4, 6, 2, 1, 5):
                    rhs = jnp.concatenate([xs_v[_RHS_AS_LHS[i], u, :, n:n + 256] for u in units], axis=0)
                    prods[i] = _dot(_as_matrix(ps_v[i, m // 2:(m + MT) // 2, :]), _as_matrix(rhs))
                for t, (i, j) in zip(_combine(prods), ((0, 0), (0, 1), (1, 0), (1, 1))):
                    rows = slice(i * HD + m, i * HD + m + MT)
                    for k in (0, 128):
                        if first:
                            t_v[(j * HD + n + k) // 128, rows, :] = t[:, k:k + 128]
                        else:
                            t_v[(j * HD + n + k) // 128, rows, :] += t[:, k:k + 128]

    x0 = [pltpu.make_async_copy(x_hbm.at[pl.ds(u * U, U)], x_v.at[pl.ds(u * U, U)], sem_s.at[u]) for u in (0, 1)]
    w22 = [pltpu.make_async_copy(wqkv_hbm.at[pl.ds(HD + h, HD // 2), pl.ds(D + HD, HD)],
                                 wk_v.at[1, 1, pl.ds(h, HD // 2)], sem_s.at[2 + h // (HD // 2)])
           for h in (0, HD // 2)]
    for cp in (x0[0], wk_cp(0, 0), *w22):
        cp.start()
    r16 = lax.broadcasted_iota(jnp.int32, (16, D), 0)
    wr = wr_ref[...].astype(F32).reshape(1, D)
    gw = gw_ref[...].astype(F32).reshape(1, D)
    rg_v[...] = jnp.where(r16 == 0, wr, jnp.where(r16 == 1, gw, 0.0)).astype(BF16)
    w22[0].wait()
    for cp in (x0[1], wk_cp(0, 1), wk_cp(1, 0)):
        cp.start()
    for cp in (w22[1], x0[0], wk_cp(0, 0)):
        cp.wait()
    put_w_terms((1, 4, 0), lambda a: wk_v.at[a // 2, a // 2])
    make_x_terms(0)
    early = [{i: proj_term(0, i) for i in (1, 4, 0)}]
    for h in (0, 1):
        route(0, h)
    for cp in (x0[1], wk_cp(0, 1), wk_cp(1, 0)):
        cp.wait()
    for c in range(1, NC):
        x_cp(c).start()
    make_x_terms(1)
    put_w_terms((3, 6, 2, 5), lambda a: wk_v.at[a // 2, a % 2])
    early.append({i: proj_term(1, i) for i in (1, 4, 0)})
    for u in range(UC):
        for n, i in enumerate((3, 6, 2, 5)):
            early[u][i] = proj_term(u, i)
            if u == 1 and n < 2:
                route(u, n)
        k_finish(u, early[u], u == 0)
    t_part(range(UC), True)
    for c in range(1, NC):
        x_cp(c).wait()
    for cp in (wq_cp, wv_cp, wo_cp) + f_cps(0):
        cp.start()

    def p1(c, carry):
        for cp in f_cps(c):
            cp.start()
        units = [c * UC + t for t in range(UC)]
        for u in units:
            make_x_terms(u)
        for t, u in enumerate(units):
            prods = {}
            for n, i in enumerate((2, 3, 0, 4, 6, 1, 5)):
                prods[i] = proj_term(u, i, True)
                if n in (2, 4):
                    route(u, n // 2 - 1)
            k_finish(t, prods, False)
        t_part(units, False)
        return carry

    lax.fori_loop(1, NC, p1, 0)

    wq_cp.wait()
    wv_cp.wait()
    wo_cp.wait()
    r = r_v[:, 0:1, :]
    tok = (lax.broadcasted_iota(jnp.int32, r.shape, 0) * UH
           + lax.broadcasted_iota(jnp.int32, r.shape, 2))
    best = jnp.max(jnp.max(jnp.where(r != r, -jnp.inf, r), axis=0), axis=1, keepdims=True)
    bidx = jnp.min(jnp.min(jnp.where(r == best, tok, S), axis=0), axis=1, keepdims=True)
    idx = jnp.where(bidx == S, 0, bidx)[0, 0]
    rsel = jnp.where(bidx == S, jnp.nan, best)
    base = pl.multiple_of((idx // 16) * 16, 16)
    sel = lax.broadcasted_iota(jnp.int32, (16, 1), 0) == idx - base
    xsel = jnp.sum(jnp.where(sel, x_v[pl.ds(base, 16), :].astype(F32), 0.0), axis=0, keepdims=True)
    xsel_v[...] = jnp.broadcast_to(xsel, (8, D))
    y_v[...] = jnp.zeros_like(y_v)

    put_w_terms(range(7), lambda a: wq_v.at[pl.ds(a // 2 * HD, HD), pl.ds(a % 2 * HD, HD)])
    z_v[...] = jnp.broadcast_to(jnp.sum(z_v[...], axis=1, keepdims=True), z_v.shape)
    same_head = ((lax.broadcasted_iota(jnp.int32, (128, 128), 0) // 16) % 4
                 == lax.broadcasted_iota(jnp.int32, (128, 128), 1) // DH)
    kvs = {}
    for o in range(0, D, 128):
        t = jnp.concatenate([
            jnp.concatenate([t_v[n, pl.ds(o + h, 32, stride=4), :] for h in range(4)], axis=0)
            for n in range(D // 128)], axis=1)
        kvs[o] = jnp.where(same_head, _dot(t.astype(BF16), wv_v[:, o:o + 128]), 0.0).astype(BF16)
    for j in range(0, HD, 128):
        for n in range(0, HD, 128):
            m = [_dot(kvs[o], wo_v[o:o + 128, h + n:h + n + 128]) for o in (j, HD + j) for h in (0, HD)]
            for i, t in enumerate(_rhs_terms(*m)):
                ms_v[i, j // 2:j // 2 + 64, n:n + 128] = _words(t[:64], t[64:])

    def ffn_steps(c):
        st = {}

        def proj(key, w_v, n, k):
            def step():
                p = _dot(xsel_v[:, k:k + HD], w_v[c, k:k + HD, n:n + 128])
                st[key, n] = p if k == 0 else st[key, n] + p
            return step

        def down(n, k):
            def step():
                if k == 0:
                    g = st['g', n]
                    st['h', n] = (g * _sigmoid(g) * st['u', n]).astype(BF16).astype(F32)
                y_v[:, k:k + HD] += _dot(st['h', n], wd_v[c, n:n + 128, k:k + HD])
            return step

        tiles = range(0, FC, 128)
        return ([proj(key, w_v, n, k) for n in tiles for key, w_v in (('g', wg_v), ('u', wu_v)) for k in (0, HD)]
                + [down(n, k) for n in tiles for k in (0, HD)])

    def unit(c, t):
        return (idx // U + 1 + c * UC + t) % NU

    def p2(c, carry):
        for cp in f_cps(c):
            cp.wait()
        steps = ffn_steps(c)

        def with_ffn(p):
            if steps:
                steps.pop(0)()
            return p

        units = [unit(c, t) for t in range(UC)]
        for t, u in enumerate(units):
            q = _combine({i: with_ffn(proj_term(u, i)) for i in (2, 3, 0, 4, 6, 1, 5)})
            pqn = []
            for qij, o in zip(q, (0, HD, 0, HD)):
                pq = _phi(qij).reshape(HD // DH, DH, UH)
                den = jnp.sum(pq * z_v[o:o + HD, :].reshape(HD // DH, DH, UH), axis=1, keepdims=True) + 1e-6
                pqn.append((pq * (1.0 / den)).reshape(HD, UH))
            for i, p in enumerate(_lhs_terms(*pqn)):
                rs_v[t, i] = p.T.astype(BF16)
        y = None
        for t, u in enumerate(units):
            if t == UC - 1:
                assert not steps
                y = y_v[:1, :] * _sigmoid(rsel)
            for n in range(0, HD, 128):
                a = _combine({i: with_ffn(_dot(rs_v[t, i], _as_matrix(ms_v[i, :, n:n + 128])))
                              for i in (0, 3, 4, 6, 2, 1, 5)})
                for aij, (i, j) in zip(a, ((0, 0), (0, 1), (1, 0), (1, 1))):
                    o = pl.multiple_of(u * U + i * UH, UH)
                    rows, cols = pl.ds(o, UH), slice(j * HD + n, j * HD + n + 128)
                    g = g_v[rows, :]
                    b = x_v[rows, cols].astype(F32)
                    upd = b * 0.0
                    if y is not None:
                        hit = lax.broadcasted_iota(jnp.int32, (UH, 128), 0) == idx - o
                        upd = upd + jnp.where(hit, y[:, cols], 0.0)
                    out_v[rows, cols] = (g * aij + (1.0 - g) * (b + upd)).astype(BF16)
                if t == UC - 1 and (n + 128) % OW == 0:
                    for cp in out_cps(c, t, u, n + 128 - OW):
                        cp.start()
            if t < UC - 1:
                for cp in out_cps(c, t, u):
                    cp.start()
        return carry

    lax.fori_loop(0, NC, p2, 0)
    for c in range(NC):
        for t in range(UC):
            for n in range(0, HD if t == UC - 1 else 1, OW):
                for cp in out_cps(c, t, unit(c, t), n):
                    cp.wait()


@jax.jit
def pallas_gated_mix__linear_attn_block__moe_arch_mod__prompt_kernel(
    A_x, A_wqkv, A_wo, B_x, B_w_r, B_w_gate, B_w_up, B_w_down, gate_w,
):
    del B_x
    hbm = pl.BlockSpec(memory_space=pl.ANY)
    vmem = pl.BlockSpec(memory_space=pltpu.VMEM)
    out = pl.pallas_call(
        _body,
        out_shape=jax.ShapeDtypeStruct((S, D), BF16),
        in_specs=[hbm, hbm, hbm, vmem, hbm, hbm, hbm, vmem],
        out_specs=hbm,
        scratch_shapes=[
            pltpu.VMEM((S, D), BF16),
            pltpu.VMEM((2, 2, HD, HD), BF16),
            pltpu.VMEM((D, D), BF16),
            pltpu.VMEM((D, D), BF16),
            pltpu.VMEM((D, D), BF16),
            pltpu.VMEM((NC, D, FC), BF16),
            pltpu.VMEM((NC, D, FC), BF16),
            pltpu.VMEM((NC, FC, D), BF16),
            pltpu.VMEM((7, NU, UH // 2, HD), U32),
            pltpu.VMEM((7, HD // 2, HD), U32),
            pltpu.VMEM((7, HD // 2, UC * UH), U32),
            pltpu.VMEM((D // 128, D, 128), F32),
            pltpu.VMEM((D, 128), F32),
            pltpu.VMEM((7, HD // 2, HD), U32),
            pltpu.VMEM((UC, 7, UH, HD), BF16),
            pltpu.VMEM((16, D), BF16),
            pltpu.VMEM((S // UH, 8, UH), F32),
            pltpu.VMEM((S, 128), F32),
            pltpu.VMEM((8, D), F32),
            pltpu.VMEM((8, D), F32),
            pltpu.VMEM((S, D), BF16),
            pltpu.SemaphoreType.DMA((NC,)),
            pltpu.SemaphoreType.DMA((7,)),
            pltpu.SemaphoreType.DMA((3, NC)),
            pltpu.SemaphoreType.DMA((NC, 1 + 2 * HD // OW)),
            pltpu.SemaphoreType.DMA((4,)),
        ],
        compiler_params=pltpu.CompilerParams(vmem_limit_bytes=100 * 1024 * 1024),
    )(A_x.reshape(S, D), A_wqkv, A_wo, B_w_r, B_w_gate, B_w_up, B_w_down, gate_w)
    return out.reshape(1, S, D)
```

```python
import jax
import jax.numpy as jnp
from jax import lax
import jax.experimental.pallas as pl
import jax.experimental.pallas.tpu as pltpu

S, D, F, DH = 2048, 1024, 3584, 32
HD = D // 2
U = 256
UH = U // 2
NU = S // U
UC = 2
NC = NU // UC
FC = F // NC
MT = 256
OW = 256
F32, BF16, U32 = jnp.float32, jnp.bfloat16, jnp.uint32
NN = (((1,), (0,)), ((), ()))
NT = (((1,), (1,)), ((), ()))


def _dot(a, b, dims=NN):
    return lax.dot_general(a, b, dims, preferred_element_type=F32)


def _phi(t):
    return jnp.where(t > 0, t + 1.0, jnp.exp(t)) + 1e-6


def _sigmoid(t):
    return 1.0 / (1.0 + jnp.exp(-t))


def _lhs_terms(a11, a12, a21, a22):
    return [a11 + a22, a21 + a22, a11, a22, a11 + a12, a21 - a11, a12 - a22]


def _rhs_terms(b11, b12, b21, b22):
    return [b11 + b22, b11, b12 - b22, b21 - b11, b22, b11 + b12, b21 + b22]


def _combine(p):
    return p[0] + p[3] - p[4] + p[6], p[2] + p[4], p[1] + p[3], p[0] - p[1] + p[2] + p[5]


_RHS_AS_LHS = (0, 2, 6, 5, 3, 4, 1)


def _as_matrix(words):
    return pltpu.bitcast(words, BF16)


def _even_odd(mat):
    words = pltpu.bitcast(mat, U32)
    return [pltpu.unpack_elementwise(words, index=i, packed_dtype=BF16, unpacked_dtype=F32) for i in (0, 1)]


def _words(even, odd):
    return pltpu.bitcast(pltpu.pack_elementwise([even, odd], packed_dtype=BF16), U32)


def _words_riffled(v):
    return jnp.concatenate([_words(v[r:r + 64], v[r + 64:r + 128]) for r in range(0, v.shape[0], 128)], axis=0)


def _body(x_hbm, wqkv_hbm, wo_hbm, wr_ref, wg_hbm, wu_hbm, wd_hbm, gw_ref, out_hbm,
          x_v, wk_v, wq_v, wv_v, wo_v, wg_v, wu_v, wd_v,
          xs_v, ws_v, ps_v, t_v, z_v, ms_v, rs_v, rg_v, r_v, g_v, xsel_v, y_v, out_v,
          sem_x, sem_w, sem_f, sem_o, sem_s):
    def x_cp(c):
        rows = pl.ds(c * UC * U, UC * U)
        return pltpu.make_async_copy(x_hbm.at[rows], x_v.at[rows], sem_x.at[c])

    def wk_cp(i, j):
        return pltpu.make_async_copy(wqkv_hbm.at[pl.ds(i * HD, HD), pl.ds(D + j * HD, HD)],
                                     wk_v.at[i, j], sem_w.at[2 * i + j])

    wq_cp = pltpu.make_async_copy(wqkv_hbm.at[:, pl.ds(0, D)], wq_v, sem_w.at[4])
    wv_cp = pltpu.make_async_copy(wqkv_hbm.at[:, pl.ds(2 * D, D)], wv_v, sem_w.at[5])
    wo_cp = pltpu.make_async_copy(wo_hbm, wo_v, sem_w.at[6])

    def f_cps(i):
        hid = pl.ds(pl.multiple_of(i * FC, 128), FC)
        return (pltpu.make_async_copy(wg_hbm.at[:, hid], wg_v.at[i], sem_f.at[0, i]),
                pltpu.make_async_copy(wu_hbm.at[:, hid], wu_v.at[i], sem_f.at[1, i]),
                pltpu.make_async_copy(wd_hbm.at[hid], wd_v.at[i], sem_f.at[2, i]))

    def out_cps(c, t, u, n=0):
        rows = pl.ds(pl.multiple_of(u * U, U), U)
        if t < UC - 1:
            return [pltpu.make_async_copy(out_v.at[rows], out_hbm.at[rows], sem_o.at[c, 0])]
        return [pltpu.make_async_copy(out_v.at[rows, pl.ds(j * HD + n, OW)], out_hbm.at[rows, pl.ds(j * HD + n, OW)],
                                      sem_o.at[c, 1 + 2 * (n // OW) + j]) for j in (0, 1)]

    def make_x_terms(u):
        for n in range(0, HD, 128):
            quads = [x_v[pl.ds(pl.multiple_of(u * U + i * UH, UH), UH), j * HD + n:j * HD + n + 128]
                     for i in (0, 1) for j in (0, 1)]
            even, odd = zip(*[_even_odd(q) for q in quads])
            for i, (e, o) in enumerate(zip(_lhs_terms(*even), _lhs_terms(*odd))):
                xs_v[i, u, :, n:n + 128] = pltpu.bitcast(quads[3 * (i - 2)], U32) if i in (2, 3) else _words(e, o)

    def put_w_terms(which, quadrant):
        pairs = {0: (0, 3, 1), 2: (1, 3, -1), 3: (2, 0, -1), 5: (0, 1, 1), 6: (2, 3, 1)}
        for r in range(0, HD, 128):
            for n in range(0, HD, 128):
                wt = [quadrant(a)[n:n + 128, r:r + 128].T for a in range(4)]
                f = [_even_odd(w) for w in wt]
                for i in which:
                    if i in pairs:
                        a, b, sign = pairs[i]
                        t = _words(*[fa + fb if sign > 0 else fa - fb for fa, fb in zip(f[a], f[b])])
                    else:
                        t = pltpu.bitcast(wt[0 if i == 1 else 3], U32)
                    ws_v[i, r // 2:r // 2 + 64, n:n + 128] = t

    def proj_term(u, i, direct=False):
        if direct and i in (2, 3):
            k = i - 2
            xt = x_v[pl.ds(pl.multiple_of(u * U + k * UH, UH), UH), k * HD:(k + 1) * HD]
        else:
            xt = _as_matrix(xs_v[i, u])
        return _dot(_as_matrix(ws_v[i]), xt, NT)

    def route(u, h):
        o = pl.multiple_of(u * U + h * UH, UH)
        rg = _dot(rg_v[...], x_v[pl.ds(o, UH), :], NT)
        r_v[2 * u + h] = rg[:8].astype(BF16).astype(F32)
        g_v[pl.ds(o, UH), :] = jnp.broadcast_to(_sigmoid(rg[1:2]), (UH, UH)).T

    def k_finish(t, prods, first):
        k11, k12, k21, k22 = [_phi(k) for k in _combine(prods)]
        if first:
            z_v[:HD, :] = k11 + k21
            z_v[HD:, :] = k12 + k22
        else:
            z_v[:HD, :] += k11 + k21
            z_v[HD:, :] += k12 + k22
        for i, p in enumerate(_lhs_terms(k11, k21, k12, k22)):
            ps_v[i, :, t * UH:(t + 1) * UH] = _words_riffled(p)

    def t_part(units, first, routed):
        routed = [(u, h) for u in routed for h in (0, 1)]
        for m in range(0, HD, MT):
            for n in range(0, HD, 256):
                prods = {}
                for i in (0, 3, 4, 6, 2, 1, 5):
                    rhs = jnp.concatenate([xs_v[_RHS_AS_LHS[i], u, :, n:n + 256] for u in units], axis=0)
                    prods[i] = _dot(_as_matrix(ps_v[i, m // 2:(m + MT) // 2, :]), _as_matrix(rhs))
                    if i == 4 and routed:
                        route(*routed.pop(0))
                for t, (i, j) in zip(_combine(prods), ((0, 0), (0, 1), (1, 0), (1, 1))):
                    rows = slice(i * HD + m, i * HD + m + MT)
                    for k in (0, 128):
                        if first:
                            t_v[(j * HD + n + k) // 128, rows, :] = t[:, k:k + 128]
                        else:
                            t_v[(j * HD + n + k) // 128, rows, :] += t[:, k:k + 128]

    x0 = [pltpu.make_async_copy(x_hbm.at[pl.ds(u * U, U)], x_v.at[pl.ds(u * U, U)], sem_s.at[u]) for u in (0, 1)]
    w22 = [pltpu.make_async_copy(wqkv_hbm.at[pl.ds(HD + h, HD // 2), pl.ds(D + HD, HD)],
                                 wk_v.at[1, 1, pl.ds(h, HD // 2)], sem_s.at[2 + h // (HD // 2)])
           for h in (0, HD // 2)]
    for cp in (x0[0], wk_cp(0, 0), *w22):
        cp.start()
    r16 = lax.broadcasted_iota(jnp.int32, (16, D), 0)
    wr = wr_ref[...].astype(F32).reshape(1, D)
    gw = gw_ref[...].astype(F32).reshape(1, D)
    rg_v[...] = jnp.where(r16 == 0, wr, jnp.where(r16 == 1, gw, 0.0)).astype(BF16)
    w22[0].wait()
    for cp in (x0[1], wk_cp(0, 1), wk_cp(1, 0)):
        cp.start()
    for cp in (w22[1], x0[0], wk_cp(0, 0)):
        cp.wait()
    put_w_terms((1, 4, 0), lambda a: wk_v.at[a // 2, a // 2])
    make_x_terms(0)
    early = [{i: proj_term(0, i) for i in (1, 4, 0)}]
    for h in (0, 1):
        route(0, h)
    for cp in (x0[1], wk_cp(0, 1), wk_cp(1, 0)):
        cp.wait()
    for c in range(1, NC):
        x_cp(c).start()
    make_x_terms(1)
    put_w_terms((3, 6, 2, 5), lambda a: wk_v.at[a // 2, a % 2])
    early.append({i: proj_term(1, i) for i in (1, 4, 0)})
    for u in range(UC):
        early[u].update({i: proj_term(u, i) for i in (3, 6, 2, 5)})
        k_finish(u, early[u], u == 0)
    t_part(range(UC), True, (1,))
    for c in range(1, NC):
        x_cp(c).wait()
    for cp in (wq_cp, wv_cp, wo_cp) + f_cps(0):
        cp.start()

    def p1(c, carry):
        for cp in f_cps(c):
            cp.start()
        units = [c * UC + t for t in range(UC)]
        for u in units:
            make_x_terms(u)
        for t, u in enumerate(units):
            k_finish(t, {i: proj_term(u, i, True) for i in (2, 3, 0, 4, 6, 1, 5)}, False)
        t_part(units, False, units)
        return carry

    lax.fori_loop(1, NC, p1, 0)

    wq_cp.wait()
    wv_cp.wait()
    wo_cp.wait()
    r = r_v[:, 0:1, :]
    tok = (lax.broadcasted_iota(jnp.int32, r.shape, 0) * UH
           + lax.broadcasted_iota(jnp.int32, r.shape, 2))
    best = jnp.max(jnp.max(jnp.where(r != r, -jnp.inf, r), axis=0), axis=1, keepdims=True)
    bidx = jnp.min(jnp.min(jnp.where(r == best, tok, S), axis=0), axis=1, keepdims=True)
    idx = jnp.where(bidx == S, 0, bidx)[0, 0]
    rsel = jnp.where(bidx == S, jnp.nan, best)
    base = pl.multiple_of((idx // 16) * 16, 16)
    sel = lax.broadcasted_iota(jnp.int32, (16, 1), 0) == idx - base
    xsel = jnp.sum(jnp.where(sel, x_v[pl.ds(base, 16), :].astype(F32), 0.0), axis=0, keepdims=True)
    xsel_v[...] = jnp.broadcast_to(xsel, (8, D))
    y_v[...] = jnp.zeros_like(y_v)

    put_w_terms(range(7), lambda a: wq_v.at[pl.ds(a // 2 * HD, HD), pl.ds(a % 2 * HD, HD)])
    z_v[...] = jnp.broadcast_to(jnp.sum(z_v[...], axis=1, keepdims=True), z_v.shape)
    same_head = ((lax.broadcasted_iota(jnp.int32, (128, 128), 0) // 16) % 4
                 == lax.broadcasted_iota(jnp.int32, (128, 128), 1) // DH)
    kvs = {}
    for o in range(0, D, 128):
        t = jnp.concatenate([
            jnp.concatenate([t_v[n, pl.ds(o + h, 32, stride=4), :] for h in range(4)], axis=0)
            for n in range(D // 128)], axis=1)
        kvs[o] = jnp.where(same_head, _dot(t.astype(BF16), wv_v[:, o:o + 128]), 0.0).astype(BF16)
    for j in range(0, HD, 128):
        for n in range(0, HD, 128):
            m = [_dot(kvs[o], wo_v[o:o + 128, h + n:h + n + 128]) for o in (j, HD + j) for h in (0, HD)]
            for i, t in enumerate(_rhs_terms(*m)):
                ms_v[i, j // 2:j // 2 + 64, n:n + 128] = _words(t[:64], t[64:])

    def ffn_steps(c):
        st = {}

        def proj(key, w_v, n, k):
            def step():
                p = _dot(xsel_v[:, k:k + HD], w_v[c, k:k + HD, n:n + 128])
                st[key, n] = p if k == 0 else st[key, n] + p
            return step

        def down(n, k):
            def step():
                if k == 0:
                    g = st['g', n]
                    st['h', n] = (g * _sigmoid(g) * st['u', n]).astype(BF16).astype(F32)
                y_v[:, k:k + HD] += _dot(st['h', n], wd_v[c, n:n + 128, k:k + HD])
            return step

        tiles = range(0, FC, 128)
        return ([proj(key, w_v, n, k) for n in tiles for key, w_v in (('g', wg_v), ('u', wu_v)) for k in (0, HD)]
                + [down(n, k) for n in tiles for k in (0, HD)])

    def unit(c, t):
        return (idx // U + 1 + c * UC + t) % NU

    def p2(c, carry):
        for cp in f_cps(c):
            cp.wait()
        steps = ffn_steps(c)

        def with_ffn(p):
            if steps:
                steps.pop(0)()
            return p

        units = [unit(c, t) for t in range(UC)]
        for t, u in enumerate(units):
            q = _combine({i: with_ffn(proj_term(u, i)) for i in (2, 3, 0, 4, 6, 1, 5)})
            pqn = []
            for qij, o in zip(q, (0, HD, 0, HD)):
                pq = _phi(qij).reshape(HD // DH, DH, UH)
                den = jnp.sum(pq * z_v[o:o + HD, :].reshape(HD // DH, DH, UH), axis=1, keepdims=True) + 1e-6
                pqn.append((pq * (1.0 / den)).reshape(HD, UH))
            for i, p in enumerate(_lhs_terms(*pqn)):
                rs_v[t, i] = p.T.astype(BF16)
        y = None
        for t, u in enumerate(units):
            if t == UC - 1:
                assert not steps
                y = y_v[:1, :] * _sigmoid(rsel)
            for n in range(0, HD, 128):
                a = _combine({i: with_ffn(_dot(rs_v[t, i], _as_matrix(ms_v[i, :, n:n + 128])))
                              for i in (0, 3, 4, 6, 2, 1, 5)})
                for aij, (i, j) in zip(a, ((0, 0), (0, 1), (1, 0), (1, 1))):
                    o = pl.multiple_of(u * U + i * UH, UH)
                    rows, cols = pl.ds(o, UH), slice(j * HD + n, j * HD + n + 128)
                    g = g_v[rows, :]
                    b = x_v[rows, cols].astype(F32)
                    upd = b * 0.0
                    if y is not None:
                        hit = lax.broadcasted_iota(jnp.int32, (UH, 128), 0) == idx - o
                        upd = upd + jnp.where(hit, y[:, cols], 0.0)
                    out_v[rows, cols] = (g * aij + (1.0 - g) * (b + upd)).astype(BF16)
                if t == UC - 1 and (n + 128) % OW == 0:
                    for cp in out_cps(c, t, u, n + 128 - OW):
                        cp.start()
            if t < UC - 1:
                for cp in out_cps(c, t, u):
                    cp.start()
        return carry

    lax.fori_loop(0, NC, p2, 0)
    for c in range(NC):
        for t in range(UC):
            for n in range(0, HD if t == UC - 1 else 1, OW):
                for cp in out_cps(c, t, unit(c, t), n):
                    cp.wait()


@jax.jit
def pallas_gated_mix__linear_attn_block__moe_arch_mod__prompt_kernel(
    A_x, A_wqkv, A_wo, B_x, B_w_r, B_w_gate, B_w_up, B_w_down, gate_w,
):
    del B_x
    hbm = pl.BlockSpec(memory_space=pl.ANY)
    vmem = pl.BlockSpec(memory_space=pltpu.VMEM)
    out = pl.pallas_call(
        _body,
        out_shape=jax.ShapeDtypeStruct((S, D), BF16),
        in_specs=[hbm, hbm, hbm, vmem, hbm, hbm, hbm, vmem],
        out_specs=hbm,
        scratch_shapes=[
            pltpu.VMEM((S, D), BF16),
            pltpu.VMEM((2, 2, HD, HD), BF16),
            pltpu.VMEM((D, D), BF16),
            pltpu.VMEM((D, D), BF16),
            pltpu.VMEM((D, D), BF16),
            pltpu.VMEM((NC, D, FC), BF16),
            pltpu.VMEM((NC, D, FC), BF16),
            pltpu.VMEM((NC, FC, D), BF16),
            pltpu.VMEM((7, NU, UH // 2, HD), U32),
            pltpu.VMEM((7, HD // 2, HD), U32),
            pltpu.VMEM((7, HD // 2, UC * UH), U32),
            pltpu.VMEM((D // 128, D + 8, 128), F32),
            pltpu.VMEM((D, 128), F32),
            pltpu.VMEM((7, HD // 2, HD), U32),
            pltpu.VMEM((UC, 7, UH, HD), BF16),
            pltpu.VMEM((16, D), BF16),
            pltpu.VMEM((S // UH, 8, UH), F32),
            pltpu.VMEM((S, 128), F32),
            pltpu.VMEM((8, D), F32),
            pltpu.VMEM((8, D), F32),
            pltpu.VMEM((S, D), BF16),
            pltpu.SemaphoreType.DMA((NC,)),
            pltpu.SemaphoreType.DMA((7,)),
            pltpu.SemaphoreType.DMA((3, NC)),
            pltpu.SemaphoreType.DMA((NC, 1 + 2 * HD // OW)),
            pltpu.SemaphoreType.DMA((4,)),
        ],
        compiler_params=pltpu.CompilerParams(vmem_limit_bytes=100 * 1024 * 1024),
    )(A_x.reshape(S, D), A_wqkv, A_wo, B_w_r, B_w_gate, B_w_up, B_w_down, gate_w)
    return out.reshape(1, S, D)
```
